```python
import jax
import jax.numpy as jnp

def _softmax(x, axis=-1):
    return jax.nn.softmax(x, axis=axis)
def _gelu(x):
    return jax.nn.gelu(x, approximate=True)
def _silu(x):
    return jax.nn.silu(x)
def _sigmoid(x):
    return jax.nn.sigmoid(x)
def _layernorm(x, axis=-1, eps=1e-5):
    m = jnp.mean(x, axis=axis, keepdims=True)
    v = jnp.var(x, axis=axis, keepdims=True)
    return (x - m) / jnp.sqrt(v + eps)
def _scatter_add(tgt, idx, src, axis=0):
    return tgt.at[idx].add(src)
def _segment_sum(src, seg, n):
    return jax.ops.segment_sum(src, seg, n)
class _Rng:
    def __init__(self, key):
        self._k = key
    def _next(self):
        self._k, sub = jax.random.split(self._k)
        return sub
    def normal(self, shape):
        return jax.random.normal(self._next(), shape, dtype=jnp.bfloat16)
    def randint(self, lo, hi, shape):
        return jax.random.randint(self._next(), shape, lo, hi, dtype=jnp.int32)
    def uniform(self, shape, lo=0.0, hi=1.0):
        return jax.random.uniform(self._next(), shape, jnp.bfloat16, lo, hi)
    def permutation(self, n):
        return jax.random.permutation(self._next(), n)


kernel_name = 'standalone__modern_conv_block_slak__vision'

def setup_inputs():
    _rng = _Rng(jax.random.key(int.from_bytes(__import__("os").urandom(4), "little")))
    _w = (lambda a: (lambda t: t.astype(jnp.bfloat16) if jnp.issubdtype(t.dtype, jnp.floating) else t)(jnp.asarray(a)))
    H = W = 384
    C = 384
    K = 1
    return {
        "x": _w((lambda *s: _rng.normal(s) * 0.05)(1, H, W, C)),
        "dw": _w((lambda *s: _rng.normal(s) * 0.05)(K, K, C)),
        "w1": _w((lambda *s: _rng.normal(s) * 0.05)(C, 4 * C)),
        "w2": _w((lambda *s: _rng.normal(s) * 0.05)(4 * C, C)),
        "grn_g": _w((lambda *s: _rng.normal(s) * 0.05)(4 * C)),
        "grn_b": _w((lambda *s: _rng.normal(s) * 0.05)(4 * C)),
    }

def reference(x, dw, w1, w2, grn_g, grn_b):
    B, H, W, C = x.shape
    K = dw.shape[0]
    pad = K // 2
    xp = jnp.pad(x, ((0,0),(pad,pad),(pad,pad),(0,0)))
    out = jnp.zeros_like(x)
    for i in range(K):
        for j in range(K):
            out = out + xp[:, i:i+H, j:j+W, :] * dw[i, j][None, None, None, :]
    h = _layernorm(out, axis=-1)
    h = _gelu(h @ w1)
    gx = jnp.sqrt((h * h).sum(axis=(1, 2), keepdims=True) + 1e-6)
    nx = gx / (gx.mean(axis=-1, keepdims=True) + 1e-6)
    h = grn_g[None, None, None, :] * (h * nx) + grn_b[None, None, None, :] + h
    return x + h @ w2
```

```python
import functools
import math

import jax
import jax.numpy as jnp
import jax.experimental.pallas as pl
import jax.experimental.pallas.tpu as pltpu

_LN_EPS = 1e-5
_GRN_EPS = 1e-6
_GA = 2.0 * math.sqrt(2.0 / math.pi)
_GB = 8.0 * math.sqrt(2.0 / math.pi) * 0.044715


def _make_kernel(*, T, TM, C, F, NB, P, R, NH, SUB1, NC1, SUB2):
    def tile_info(tile):
        q = tile // P
        r = tile % P
        is_res = r < R
        ridx = q * R + r
        hidx = q * (P - R) + (r - R)
        slot = jnp.where(is_res, NB + ridx, hidx % NB)
        return is_res, hidx, slot

    def kernel(x_ref, dw_ref, w1_ref, w2_ref, g_ref, b_ref,
               o_ref, hbuf_ref,
               hv_ref, acc_ref, w2s_ref, bias_ref, sem):
        phase = pl.program_id(0)
        step = pl.program_id(1)

        def write_copy(hidx, slot):
            return pltpu.make_async_copy(hv_ref.at[slot], hbuf_ref.at[hidx], sem.at[slot])

        def read_copy(hidx, slot):
            return pltpu.make_async_copy(hbuf_ref.at[hidx], hv_ref.at[slot], sem.at[slot])

        @pl.when(phase == 0)
        def _phase0():
            is_res, hidx, slot = tile_info(step)

            @pl.when(step == 0)
            def _():
                acc_ref[...] = jnp.zeros_like(acc_ref)

            @pl.when(jnp.logical_and(jnp.logical_not(is_res), hidx >= NB))
            def _():
                write_copy(hidx - NB, slot).wait()

            dw = dw_ref[...].astype(jnp.float32)

            def sub_body(si, carry):
                r0 = pl.multiple_of(si * SUB1, SUB1)
                xs = x_ref[pl.ds(r0, SUB1), :].astype(jnp.float32) * dw
                m = jnp.mean(xs, axis=-1, keepdims=True)
                xc = xs - m
                v = jnp.mean(xc * xc, axis=-1, keepdims=True)
                xn = (xc * (0.5 * lax_rsqrt(v + _LN_EPS))).astype(jnp.bfloat16)
                for n in range(F // NC1):
                    cs = slice(n * NC1, (n + 1) * NC1)
                    y = jnp.dot(xn, w1_ref[:, cs], preferred_element_type=jnp.float32)
                    t = jnp.tanh(y * (_GA + _GB * (y * y)))
                    g = y + y * t
                    gg = (g * g).reshape(SUB1 // 8, 8, NC1)
                    acc_ref[:, cs] += jnp.sum(gg, axis=0)
                    hv_ref[slot, pl.ds(r0, SUB1), cs] = g.astype(jnp.bfloat16)
                return carry

            jax.lax.fori_loop(0, TM // SUB1, sub_body, 0)

            @pl.when(jnp.logical_and(jnp.logical_not(is_res), hidx < NH - NB))
            def _():
                write_copy(hidx, slot).start()

        @pl.when(phase == 1)
        def _phase1():
            tile = T - 1 - step
            is_res, hidx, slot = tile_info(tile)

            @pl.when(step == 0)
            def _():
                ss = jnp.sum(acc_ref[...], axis=0, keepdims=True)
                gx = jnp.sqrt(ss + _GRN_EPS)
                nx = gx / (jnp.mean(gx, axis=-1, keepdims=True) + _GRN_EPS)
                s = g_ref[...].astype(jnp.float32) * nx + 1.0
                st = jnp.transpose(jnp.broadcast_to(s, (128, F)))
                for j in range(C // 128):
                    cs = slice(j * 128, (j + 1) * 128)
                    w2s_ref[:, cs] = (w2_ref[:, cs].astype(jnp.float32) * st).astype(jnp.bfloat16)
                bb = jnp.broadcast_to(b_ref[...], (16, F))
                bias_ref[...] = jnp.dot(bb, w2_ref[...], preferred_element_type=jnp.float32)[:8]

            @pl.when(jnp.logical_and(jnp.logical_not(is_res), hidx < NH - NB))
            def _():
                read_copy(hidx, slot).wait()

            bias = bias_ref[0:1, :]

            def sub_body(si, carry):
                r0 = pl.multiple_of(si * SUB2, SUB2)
                hs = hv_ref[slot, pl.ds(r0, SUB2), :]
                y = jnp.dot(hs, w2s_ref[...], preferred_element_type=jnp.float32)
                y = y + bias + x_ref[pl.ds(r0, SUB2), :].astype(jnp.float32)
                o_ref[pl.ds(r0, SUB2), :] = y.astype(o_ref.dtype)
                return carry

            jax.lax.fori_loop(0, TM // SUB2, sub_body, 0)

            @pl.when(jnp.logical_and(jnp.logical_not(is_res), hidx >= NB))
            def _():
                read_copy(hidx - NB, slot).start()

    return kernel


def lax_rsqrt(v):
    return jax.lax.rsqrt(v)


def _run(x, dw, w1, w2, grn_g, grn_b, *, TM=1024, NB=4, P=9, R=2, SUB1=256, NC1=512,
         SUB2=512, VMEM_MB=120):
    B, H, W, C = x.shape
    F = w1.shape[1]
    N = B * H * W
    T = N // TM
    assert N % TM == 0 and T % P == 0
    NR = (T // P) * R
    NH = T - NR
    assert NH > NB

    x2 = x.reshape(N, C)
    dw2 = dw.reshape(1, C)
    g2 = grn_g.reshape(1, F)
    b2 = grn_b.reshape(1, F)

    kernel = _make_kernel(T=T, TM=TM, C=C, F=F, NB=NB, P=P, R=R, NH=NH,
                          SUB1=SUB1, NC1=NC1, SUB2=SUB2)

    def tok_map(p, i):
        return (i + p * (T - 1 - 2 * i), 0)

    def out_map(p, i):
        return (T - 1 - p * i, 0)

    const = lambda p, i: (0, 0)

    out, _ = pl.pallas_call(
        kernel,
        grid=(2, T),
        in_specs=[
            pl.BlockSpec((TM, C), tok_map),
            pl.BlockSpec((1, C), const),
            pl.BlockSpec((C, F), const),
            pl.BlockSpec((F, C), const),
            pl.BlockSpec((1, F), const),
            pl.BlockSpec((1, F), const),
        ],
        out_specs=[
            pl.BlockSpec((TM, C), out_map),
            pl.BlockSpec(memory_space=pl.ANY),
        ],
        out_shape=[
            jax.ShapeDtypeStruct((N, C), x.dtype),
            jax.ShapeDtypeStruct((NH - NB, TM, F), jnp.bfloat16),
        ],
        scratch_shapes=[
            pltpu.VMEM((NB + NR, TM, F), jnp.bfloat16),
            pltpu.VMEM((8, F), jnp.float32),
            pltpu.VMEM((F, C), jnp.bfloat16),
            pltpu.VMEM((8, C), jnp.float32),
            pltpu.SemaphoreType.DMA((NB,)),
        ],
        compiler_params=pltpu.CompilerParams(
            dimension_semantics=("arbitrary", "arbitrary"),
            vmem_limit_bytes=VMEM_MB * 1024 * 1024,
        ),
    )(x2, dw2, w1, w2, g2, b2)
    return out.reshape(B, H, W, C)


@jax.jit
def pallas_standalone__modern_conv_block_slak__vision_kernel(
    x: jax.Array,
    dw: jax.Array,
    w1: jax.Array,
    w2: jax.Array,
    grn_g: jax.Array,
    grn_b: jax.Array,
):
    return _run(x, dw, w1, w2, grn_g, grn_b)
```

```python
import functools
import math

import jax
import jax.numpy as jnp
import jax.experimental.pallas as pl
import jax.experimental.pallas.tpu as pltpu

_LN_EPS = 1e-5
_GRN_EPS = 1e-6
_GA = 2.0 * math.sqrt(2.0 / math.pi)
_GB = 8.0 * math.sqrt(2.0 / math.pi) * 0.044715


def _make_kernel(*, T, TM, C, F, NB, NR, NH, SUB1, NC1, SUB2, UNR1, UNR2, NODMA=0, ONLY=-1, PRIO=0):
    def tile_info(tile):
        ridx = (tile * NR) // T
        is_res = ((tile + 1) * NR) // T > ridx
        hidx = tile - ridx
        slot = jnp.where(is_res, NB + ridx, hidx % NB)
        return is_res, hidx, slot

    def kernel(x_ref, dw_ref, w1_ref, w2_ref, g_ref, b_ref,
               o_ref, hbuf_ref,
               hv_ref, acc_ref, w2s_ref, bias_ref, sem):
        phase = pl.program_id(0) if ONLY < 0 else ONLY
        step = pl.program_id(1)

        class _Nop:
            def start(self, priority=0): pass
            def wait(self): pass

        def write_copy(hidx, slot):
            if NODMA: return _Nop()
            return pltpu.make_async_copy(hv_ref.at[slot], hbuf_ref.at[hidx], sem.at[slot])

        def read_copy(hidx, slot):
            if NODMA: return _Nop()
            return pltpu.make_async_copy(hbuf_ref.at[hidx], hv_ref.at[slot], sem.at[slot])

        @pl.when(jnp.equal(phase, 0))
        def _phase0():
            is_res, hidx, slot = tile_info(step)

            @pl.when(step == 0)
            def _():
                acc_ref[...] = jnp.zeros_like(acc_ref)

            @pl.when(jnp.logical_and(jnp.logical_not(is_res), hidx >= NB))
            def _():
                write_copy(hidx - NB, slot).wait()

            dw = dw_ref[...].astype(jnp.float32)

            def sub_body(si, carry):
                r0 = pl.multiple_of(si * SUB1, SUB1)
                xs = x_ref[pl.ds(r0, SUB1), :].astype(jnp.float32) * dw
                m = jnp.mean(xs, axis=-1, keepdims=True)
                xc = xs - m
                v = jnp.mean(xc * xc, axis=-1, keepdims=True)
                xn = (xc * (0.5 * lax_rsqrt(v + _LN_EPS))).astype(jnp.bfloat16)
                for n in range(F // NC1):
                    cs = slice(n * NC1, (n + 1) * NC1)
                    y = jnp.dot(xn, w1_ref[:, cs], preferred_element_type=jnp.float32)
                    t = jnp.tanh(y * (_GA + _GB * (y * y)))
                    g = y + y * t
                    gg = (g * g).reshape(SUB1 // 8, 8, NC1)
                    acc_ref[:, cs] += jnp.sum(gg, axis=0)
                    hv_ref[slot, pl.ds(r0, SUB1), cs] = g.astype(jnp.bfloat16)
                return carry

            jax.lax.fori_loop(0, TM // SUB1, sub_body, 0, unroll=UNR1)

            @pl.when(jnp.logical_and(jnp.logical_not(is_res), hidx < NH - NB))
            def _():
                write_copy(hidx, slot).start(priority=PRIO)

        @pl.when(jnp.equal(phase, 1))
        def _phase1():
            tile = T - 1 - step
            is_res, hidx, slot = tile_info(tile)

            @pl.when(step == 0)
            def _():
                ss = jnp.sum(acc_ref[...], axis=0, keepdims=True)
                gx = jnp.sqrt(ss + _GRN_EPS)
                nx = gx / (jnp.mean(gx, axis=-1, keepdims=True) + _GRN_EPS)
                s = g_ref[...].astype(jnp.float32) * nx + 1.0
                st = jnp.transpose(jnp.broadcast_to(s, (128, F)))
                for j in range(C // 128):
                    cs = slice(j * 128, (j + 1) * 128)
                    w2s_ref[:, cs] = (w2_ref[:, cs].astype(jnp.float32) * st).astype(jnp.bfloat16)
                bb = jnp.broadcast_to(b_ref[...], (16, F))
                bias_ref[...] = jnp.dot(bb, w2_ref[...], preferred_element_type=jnp.float32)[:8]

            @pl.when(jnp.logical_and(jnp.logical_not(is_res), hidx < NH - NB))
            def _():
                read_copy(hidx, slot).wait()

            bias = bias_ref[0:1, :]

            def sub_body(si, carry):
                r0 = pl.multiple_of(si * SUB2, SUB2)
                hs = hv_ref[slot, pl.ds(r0, SUB2), :]
                y = jnp.dot(hs, w2s_ref[...], preferred_element_type=jnp.float32)
                y = y + bias + x_ref[pl.ds(r0, SUB2), :].astype(jnp.float32)
                o_ref[pl.ds(r0, SUB2), :] = y.astype(o_ref.dtype)
                return carry

            jax.lax.fori_loop(0, TM // SUB2, sub_body, 0, unroll=UNR2)

            @pl.when(jnp.logical_and(jnp.logical_not(is_res), hidx >= NB))
            def _():
                read_copy(hidx - NB, slot).start(priority=PRIO)

    return kernel


def lax_rsqrt(v):
    return jax.lax.rsqrt(v)


def _run(x, dw, w1, w2, grn_g, grn_b, *, TM=3072, NB=3, NR=8, SUB1=64, NC1=512,
         SUB2=1024, UNR1=48, UNR2=3, VMEM_MB=120, NODMA=0, ONLY=-1, PRIO=1, XBUF=2):
    B, H, W, C = x.shape
    F = w1.shape[1]
    N = B * H * W
    T = N // TM
    assert N % TM == 0
    NH = T - NR
    assert NH > NB

    x2 = x.reshape(N, C)
    dw2 = dw.reshape(1, C)
    g2 = grn_g.reshape(1, F)
    b2 = grn_b.reshape(1, F)

    kernel = _make_kernel(T=T, TM=TM, C=C, F=F, NB=NB, NR=NR, NH=NH,
                          SUB1=SUB1, NC1=NC1, SUB2=SUB2, UNR1=UNR1, UNR2=UNR2, NODMA=NODMA, ONLY=ONLY, PRIO=PRIO)

    def tok_map(p, i):
        p = p if ONLY < 0 else ONLY
        return (i + p * (T - 1 - 2 * i), 0)

    def out_map(p, i):
        p = p if ONLY < 0 else ONLY
        return (T - 1 - p * i, 0)

    const = lambda p, i: (0, 0)

    out, _ = pl.pallas_call(
        kernel,
        grid=(2 if ONLY < 0 else 1, T),
        in_specs=[
            pl.BlockSpec((TM, C), tok_map, pipeline_mode=pl.Buffered(XBUF)),
            pl.BlockSpec((1, C), const),
            pl.BlockSpec((C, F), const),
            pl.BlockSpec((F, C), const),
            pl.BlockSpec((1, F), const),
            pl.BlockSpec((1, F), const),
        ],
        out_specs=[
            pl.BlockSpec((TM, C), out_map),
            pl.BlockSpec(memory_space=pl.ANY),
        ],
        out_shape=[
            jax.ShapeDtypeStruct((N, C), x.dtype),
            jax.ShapeDtypeStruct((NH - NB, TM, F), jnp.bfloat16),
        ],
        scratch_shapes=[
            pltpu.VMEM((NB + NR, TM, F), jnp.bfloat16),
            pltpu.VMEM((8, F), jnp.float32),
            pltpu.VMEM((F, C), jnp.bfloat16),
            pltpu.VMEM((8, C), jnp.float32),
            pltpu.SemaphoreType.DMA((NB,)),
        ],
        compiler_params=pltpu.CompilerParams(
            dimension_semantics=("arbitrary", "arbitrary"),
            vmem_limit_bytes=VMEM_MB * 1024 * 1024,
        ),
    )(x2, dw2, w1, w2, g2, b2)
    return out.reshape(B, H, W, C)


@jax.jit
def pallas_standalone__modern_conv_block_slak__vision_kernel(
    x: jax.Array,
    dw: jax.Array,
    w1: jax.Array,
    w2: jax.Array,
    grn_g: jax.Array,
    grn_b: jax.Array,
):
    return _run(x, dw, w1, w2, grn_g, grn_b)
```

```python
import math

import jax
import jax.numpy as jnp
import jax.experimental.pallas as pl
import jax.experimental.pallas.tpu as pltpu

_LN_EPS = 1e-5
_GRN_EPS = 1e-6
_GA = 2.0 * math.sqrt(2.0 / math.pi)
_GB = 8.0 * math.sqrt(2.0 / math.pi) * 0.044715
_ALPHA = _GB ** (-1.0 / 3.0)
_GZ = _GA * _ALPHA
_NX = 3
_KT = 128
_BF = jnp.bfloat16
_F32 = jnp.float32
_U32 = jnp.uint32


def _pack(v):
    return pltpu.bitcast(v.astype(_BF), _U32)


def _unpack(u):
    return pltpu.bitcast(u, _BF)


def _dot(a, b):
    return jnp.dot(a, b, preferred_element_type=_F32)


def _make_kernel(*, T, TM, C, F, S, SUB1, SUB2, PRIO):
    KT = _KT
    FH = F // 2
    NQ = FH // KT
    H1 = SUB1 // 2
    H2 = SUB2 // 2
    NCH = TM // SUB2

    def inc_mod(v, m):
        return jnp.where(v + 1 == m, 0, v + 1)

    def dec_mod(v, m):
        return jnp.where(v == 0, m - 1, v - 1)

    def kernel(x_hbm, dw_hbm, w1_hbm, w2_hbm, g_hbm, b_hbm,
               o_hbm, hbuf_hbm,
               xv, hv, w1v, w2v, wc, lk, acc_ref, bias_ref, dwv, gv, bv,
               xsem, osem, hsem, wsem):

        def x_copy(tile, s):
            return pltpu.make_async_copy(x_hbm.at[pl.ds(tile * TM, TM)], xv.at[s], xsem.at[s])

        def o_copy(tile, s, c):
            r = c * SUB2
            return pltpu.make_async_copy(xv.at[s, pl.ds(r, SUB2)],
                                         o_hbm.at[pl.ds(tile * TM + r, SUB2)], osem.at[s])

        def h_write(tile, slot):
            return pltpu.make_async_copy(hv.at[slot], hbuf_hbm.at[tile], hsem.at[slot])

        def h_read(tile, slot, c):
            rows = pl.ds(c * SUB2, SUB2)
            return pltpu.make_async_copy(hbuf_hbm.at[tile, :, rows, :], hv.at[slot, :, rows, :],
                                         hsem.at[slot])

        w1_copy = pltpu.make_async_copy(w1_hbm, w1v, wsem.at[0])
        w2_copy = pltpu.make_async_copy(w2_hbm, w2v, wsem.at[1])
        dw_copy = pltpu.make_async_copy(dw_hbm, dwv, wsem.at[2])
        g_copy = pltpu.make_async_copy(g_hbm, gv, wsem.at[3])
        b_copy = pltpu.make_async_copy(b_hbm, bv, wsem.at[4])

        dw_copy.start()
        w1_copy.start()
        x_copy(0, 0).start()

        acc_ref[...] = jnp.zeros_like(acc_ref)

        w1_copy.wait()
        b11 = w1v[0:KT, 0:FH].astype(_F32)
        b12 = w1v[0:KT, FH:F].astype(_F32)
        b21 = w1v[KT:2 * KT, 0:FH].astype(_F32)
        b22 = w1v[KT:2 * KT, FH:F].astype(_F32)
        t1 = b12 - b11
        t2 = b22 - t1
        combos = (b11, b21, b22, t2 - b21, t1, t2, b22 - b12,
                  w1v[2 * KT:3 * KT, 0:FH], w1v[2 * KT:3 * KT, FH:F])
        for i, cmb in enumerate(combos):
            for q in range(NQ):
                wc[i * NQ + q] = _pack(cmb[:, q * KT:(q + 1) * KT])

        dw_copy.wait()
        dw = dwv[0].astype(_F32)

        def prep(xs):
            xs = xs.astype(_F32) * dw
            m = jnp.mean(xs, axis=-1, keepdims=True)
            xc = xs - m
            v = jnp.mean(xc * xc, axis=-1, keepdims=True)
            xn = xc * jnp.exp(math.log(0.5 / _ALPHA) - 0.5 * jnp.log(v + _LN_EPS))
            a11, a12, a13 = xn[:H1, 0:KT], xn[:H1, KT:2 * KT], xn[:H1, 2 * KT:3 * KT]
            a21, a22, a23 = xn[H1:, 0:KT], xn[H1:, KT:2 * KT], xn[H1:, 2 * KT:3 * KT]
            s1 = a21 + a22
            s2 = s1 - a11
            ops = (a11, a12, a12 - s2, a22, s1, s2, a11 - a21, a13, a23)
            return [o.astype(_BF) for o in ops]

        x_copy(0, 0).wait()
        x_copy(1, 1).start()
        w2_copy.start(priority=PRIO)
        g_copy.start()
        b_copy.start()
        for i, o in enumerate(prep(xv[0, 0:SUB1, :])):
            lk[i] = pltpu.bitcast(o, _U32)

        def gelu_store(z, slot, r0, q):
            rows = z.shape[0]
            g = z + z * jnp.tanh(z * (_GZ + z * z))
            gg = (g * g).reshape(rows // 8, 8, KT)
            acc_ref[:, q * KT:(q + 1) * KT] += jnp.sum(gg, axis=0)
            hv[slot, q, r0:r0 + rows, :] = g.astype(_BF)

        def phase0(t, carry):
            slot, xs_cur = carry
            xs_n1 = inc_mod(xs_cur, _NX)
            xs_n2 = inc_mod(xs_n1, _NX)

            @pl.when(t + 1 < T)
            def _():
                x_copy(t + 1, xs_n1).wait()

            @pl.when(t + 2 < T)
            def _():
                x_copy(t + 2, xs_n2).start()

            @pl.when(t >= S)
            def _():
                h_write(t - S, slot).wait()

            for si in range(TM // SUB1):
                r0 = si * SUB1
                if si == 0:
                    L = [_unpack(lk[i]) for i in range(lk.shape[0])]
                else:
                    L = prep(xv[xs_cur, r0:r0 + SUB1, :])
                for q in range(NQ):
                    W = lambda i: _unpack(wc[i * NQ + q])
                    p1 = _dot(L[0], W(0))
                    gelu_store(p1 + _dot(L[1], W(1)) + _dot(L[7], W(7)), slot, r0, q)
                    u2 = p1 + _dot(L[5], W(5))
                    p5 = _dot(L[4], W(4))
                    gelu_store(u2 + p5 + _dot(L[2], W(2)) + _dot(L[7], W(8)), slot, r0, NQ + q)
                    u3 = u2 + _dot(L[6], W(6))
                    gelu_store(u3 + p5 + _dot(L[8], W(8)), slot, r0 + H1, NQ + q)
                    gelu_store(u3 - _dot(L[3], W(3)) + _dot(L[8], W(7)), slot, r0 + H1, q)

            xs_nxt = jnp.where(t + 1 < T, xs_n1, xs_cur)
            for i, o in enumerate(prep(xv[xs_nxt, 0:SUB1, :])):
                lk[i] = pltpu.bitcast(o, _U32)

            @pl.when(t < T - S)
            def _():
                h_write(t, slot).start(priority=PRIO)

            return inc_mod(slot, S), xs_n1

        i32 = jnp.int32
        jax.lax.fori_loop(0, T, phase0, (i32(0), i32(0)))

        w2_copy.wait()
        g_copy.wait()
        b_copy.wait()
        ss = jnp.sum(acc_ref[...], axis=0, keepdims=True)
        gx = jnp.sqrt(ss * (_ALPHA * _ALPHA) + _GRN_EPS)
        nx = gx / (jnp.mean(gx, axis=-1, keepdims=True) + _GRN_EPS)
        s = (gv[...].reshape(1, F).astype(_F32) * nx + 1.0) * _ALPHA
        st = jnp.transpose(jnp.broadcast_to(s, (128, F)))
        ws = lambda r, c: (w2v[r * FH:(r + 1) * FH, c * KT:(c + 1) * KT].astype(_F32)
                           * st[r * FH:(r + 1) * FH])
        b11, b12, b21, b22 = ws(0, 0), ws(0, 1), ws(1, 0), ws(1, 1)
        combos = (b11 + b22, b11, b22, b11 + b12, b21 + b22,
                  b12 - b22, ws(0, 2), b21 - b11, ws(1, 2))
        for i, cmb in enumerate(combos):
            for q in range(NQ):
                wc[i * NQ + q] = _pack(cmb[q * KT:(q + 1) * KT, :])
        bb = jnp.broadcast_to(bv[...].reshape(1, F), (16, F))
        bias_ref[...] = _dot(bb, w2v[...])[:8]

        def phase1(j, carry):
            tile = T - 1 - j
            slot, xs_cur = carry
            xs_nxt = dec_mod(xs_cur, _NX)

            @pl.when(j >= S)
            def _():
                for c in range(NCH):
                    h_read(tile, slot, c).wait()

            @pl.when(j >= _NX)
            def _():
                x_copy(tile, xs_cur).wait()

            @pl.when(j >= _NX - 1)
            def _():
                for c in range(NCH):
                    o_copy(tile + _NX - 1, xs_nxt, c).wait()

            @pl.when(jnp.logical_and(j >= _NX - 1, tile >= 1))
            def _():
                x_copy(tile - 1, xs_nxt).start()

            bias = bias_ref[0:1, :]
            for si in range(NCH):
                r0 = si * SUB2
                rt, rb = r0, r0 + H2
                ld = lambda rr, q0: jnp.concatenate(
                    [hv[slot, q0 + q, rr:rr + H2, :] for q in range(NQ)], axis=1)
                fl = lambda rr, q0: ld(rr, q0).astype(_F32)
                W1 = lambda i: wc[i * NQ:(i + 1) * NQ].reshape(NQ * (KT // 2), KT)
                W = lambda i, n=1: _unpack(jnp.concatenate([W1(i + u) for u in range(n)], axis=1))
                d3 = _dot(ld(rt, 0), W(5, 2))
                d4 = _dot(ld(rb, NQ), W(7, 2))
                e12 = _dot(ld(rt, NQ), W(8))
                e21 = _dot(ld(rb, 0), W(6))
                m5 = _dot((fl(rt, 0) + fl(rt, NQ)).astype(_BF), W(2))
                m2 = _dot((fl(rb, 0) + fl(rb, NQ)).astype(_BF), W(1))
                m1 = _dot((fl(rt, 0) + fl(rb, NQ)).astype(_BF), W(0))
                m6 = _dot((fl(rb, 0) - fl(rt, 0)).astype(_BF), W(3))
                m7 = _dot((fl(rt, NQ) - fl(rb, NQ)).astype(_BF), W(4))
                m3, e11 = d3[:, :KT], d3[:, KT:]
                m4, e22 = d4[:, :KT], d4[:, KT:]
                yt = jnp.concatenate([m1 + m4 - m5 + m7, m3 + m5, e11 + e12], axis=1)
                yb = jnp.concatenate([m2 + m4, m1 - m2 + m3 + m6, e21 + e22], axis=1)
                for y, rr in ((yt, rt), (yb, rb)):
                    y = y + bias + xv[xs_cur, rr:rr + H2, :].astype(_F32)
                    xv[xs_cur, rr:rr + H2, :] = y.astype(xv.dtype)
                o_copy(tile, xs_cur, si).start()

                @pl.when(tile >= S)
                def _():
                    h_read(tile - S, slot, si).start(priority=PRIO)

            return dec_mod(slot, S), xs_nxt

        jax.lax.fori_loop(0, T, phase1, (i32((T - 1) % S), i32((T - 1) % _NX)))

        for tile in range(_NX - 2, -1, -1):
            for c in range(NCH):
                o_copy(tile, tile % _NX, c).wait()

    return kernel


def _run(x, dw, w1, w2, grn_g, grn_b, *, TM=3072, S=12, SUB1=128, SUB2=1024,
         VMEM_MB=127, PRIO=1, NOBC=1):
    B, H, W, C = x.shape
    F = w1.shape[1]
    N = B * H * W
    T = N // TM
    assert N % TM == 0 and T > S and T >= 3

    x2 = x.reshape(N, C)
    kernel = _make_kernel(T=T, TM=TM, C=C, F=F, S=S, SUB1=SUB1, SUB2=SUB2, PRIO=PRIO)
    any_spec = pl.BlockSpec(memory_space=pl.ANY)
    out, _ = pl.pallas_call(
        kernel,
        in_specs=[any_spec] * 6,
        out_specs=[any_spec, any_spec],
        out_shape=[
            jax.ShapeDtypeStruct((N, C), x.dtype),
            jax.ShapeDtypeStruct((T - S, F // 128, TM, 128), _BF),
        ],
        scratch_shapes=[
            pltpu.VMEM((_NX, TM, C), _BF),
            pltpu.VMEM((S, F // 128, TM, 128), _BF),
            pltpu.VMEM((C, F), _BF),
            pltpu.VMEM((F, C), _BF),
            pltpu.VMEM((54, 64, 128), _U32),
            pltpu.VMEM((9, SUB1 // 4, 128), _U32),
            pltpu.VMEM((8, F), _F32),
            pltpu.VMEM((8, C), _F32),
            pltpu.VMEM((1, 1, C), _BF),
            pltpu.VMEM((F,), _BF),
            pltpu.VMEM((F,), _BF),
            pltpu.SemaphoreType.DMA((_NX,)),
            pltpu.SemaphoreType.DMA((_NX,)),
            pltpu.SemaphoreType.DMA((S,)),
            pltpu.SemaphoreType.DMA((5,)),
        ],
        compiler_params=pltpu.CompilerParams(
            vmem_limit_bytes=VMEM_MB * 1024 * 1024,
            disable_bounds_checks=bool(NOBC),
        ),
    )(x2, dw, w1, w2, grn_g, grn_b)
    return out.reshape(B, H, W, C)


@jax.jit
def pallas_standalone__modern_conv_block_slak__vision_kernel(
    x: jax.Array,
    dw: jax.Array,
    w1: jax.Array,
    w2: jax.Array,
    grn_g: jax.Array,
    grn_b: jax.Array,
):
    return _run(x, dw, w1, w2, grn_g, grn_b)
```

```python
import math

import jax
import jax.numpy as jnp
import jax.experimental.pallas as pl
import jax.experimental.pallas.tpu as pltpu

_LN_EPS = 1e-5
_GRN_EPS = 1e-6
_GA = 2.0 * math.sqrt(2.0 / math.pi)
_GB = 8.0 * math.sqrt(2.0 / math.pi) * 0.044715
_ALPHA = _GB ** (-1.0 / 3.0)
_GZ = _GA * _ALPHA
_KT = 128
_BF = jnp.bfloat16
_F32 = jnp.float32
_U32 = jnp.uint32

_HK_U = (
    ((1, 1, 1),),
    ((1, 0, 0), (1, 1, 1)),
    ((1, 0, 0), (-1, 1, 0), (1, 1, 2)),
    ((1, 0, 1), (-1, 0, 2), (-1, 1, 1), (1, 1, 2)),
    ((1, 1, 0), (1, 1, 1)),
    ((1, 0, 1), (-1, 0, 2), (-1, 1, 1)),
    ((1, 1, 0), (-1, 0, 0)),
    ((1, 0, 2),),
    ((1, 0, 1), (-1, 0, 2)),
    ((1, 1, 2),),
    ((1, 0, 2), (-1, 0, 0), (1, 1, 0), (-1, 1, 2)),
    ((1, 0, 0), (1, 0, 1)),
    ((1, 1, 0), (-1, 1, 2)),
    ((1, 1, 1), (-1, 0, 1)),
    ((1, 0, 0),),
)
_NP = len(_HK_U)


def _hk_a(a11, a12, a13, a21, a22, a23):
    d1 = a12 - a13
    d2 = d1 - a22
    e1 = a21 - a23
    l2 = a11 - e1
    return (a22, a11 + a22, l2, d2 + a23, a21 + a22, d2, a21 - a11, a13, d1, a23,
            a13 - l2, a11 + a12, e1, a22 - a12, a11)


def _hk_b(b):
    return (
        b(2, 3) - b(1, 3) - b(2, 2),
        b(1, 3) - b(2, 1),
        b(1, 2) - b(3, 1),
        b(3, 3),
        b(1, 3),
        -b(2, 2) - b(3, 3),
        b(1, 1) - b(1, 3) + b(3, 1),
        b(2, 2) + b(3, 1) + b(3, 2),
        b(2, 2),
        b(1, 2) + b(3, 2) - b(3, 3),
        b(3, 1),
        b(2, 1),
        b(1, 2),
        b(2, 1) - b(2, 3) - b(3, 3),
        b(1, 1) + b(1, 2) - b(2, 1),
    )


def _hk_c(P, emit):
    q8 = P(8)
    a = P(5) + q8
    b = a + P(3)
    p0 = P(0)
    p4 = P(4)
    emit(1, 2, b + p0 + p4)
    a = a + p0
    p12 = P(12)
    emit(1, 1, b + P(9) + p12)
    d = P(2) + p12
    p10 = P(10)
    emit(0, 1, d + q8 + P(7) - p10)
    e = P(14) - d
    p11 = P(11)
    emit(0, 0, e + p10 + p11)
    p1 = P(1)
    emit(0, 2, a + p11 + p1 + P(13))
    emit(1, 0, e + p4 - p1 + P(6))


def _pack(v):
    return pltpu.bitcast(v.astype(_BF), _U32)


def _unpack(u):
    return pltpu.bitcast(u, _BF)


def _dot(a, b):
    return jnp.dot(a, b, preferred_element_type=_F32)


def _make_kernel(*, T, TM, C, F, S, NX, SUB1, SUB2, RB, DROP, PRIO):
    KT = _KT
    H1 = SUB1 // 2
    H2 = SUB2 // 2
    NCH = TM // SUB2
    NS1 = TM // SUB1
    N3 = F // (3 * KT)

    def inc_mod(v, m):
        return jnp.where(v + 1 == m, 0, v + 1)

    def dec_mod(v, m):
        return jnp.where(v == 0, m - 1, v - 1)

    def kept(t):
        k = t >= 0
        for d in DROP:
            k = jnp.logical_and(k, t != d)
        return k

    def hidx(t):
        i = t
        for d in DROP:
            i = i - (t > d).astype(jnp.int32)
        return i

    def kernel(x_hbm, dw_hbm, w1_hbm, w2_hbm, g_hbm, b_hbm,
               o_hbm, hbuf_hbm,
               xv, hv, w1v, w2v, wc1, wc2, lk, acc_ref, bias_ref, dwv, gv, bv,
               xsem, osem, hsem, wsem):

        def x_copy(tile, s):
            return pltpu.make_async_copy(x_hbm.at[pl.ds(tile * TM, TM)], xv.at[s], xsem.at[s])

        def o_copy(tile, s, c):
            r = c * SUB2
            return pltpu.make_async_copy(xv.at[s, pl.ds(r, SUB2)],
                                         o_hbm.at[pl.ds(tile * TM + r, SUB2)], osem.at[s])

        def h_write(tile, slot):
            return pltpu.make_async_copy(hv.at[slot], hbuf_hbm.at[hidx(tile)], hsem.at[slot])

        def h_read(tile, slot, c):
            rows = pl.ds(c * SUB2, SUB2)
            return pltpu.make_async_copy(hbuf_hbm.at[hidx(tile), :, rows, :],
                                         hv.at[slot, :, rows, :], hsem.at[slot])

        w1_copy = pltpu.make_async_copy(w1_hbm, w1v, wsem.at[0])
        w2_copy = pltpu.make_async_copy(w2_hbm, w2v, wsem.at[1])
        dw_copy = pltpu.make_async_copy(dw_hbm, dwv, wsem.at[2])
        g_copy = pltpu.make_async_copy(g_hbm, gv, wsem.at[3])
        b_copy = pltpu.make_async_copy(b_hbm, bv, wsem.at[4])

        dw_copy.start()
        w1_copy.start()
        x_copy(0, 0).start()

        acc_ref[...] = jnp.zeros_like(acc_ref)

        w1_copy.wait()
        for q in range(N3):
            b = lambda l, j: w1v[(l - 1) * KT:l * KT,
                                 ((j - 1) * N3 + q) * KT:((j - 1) * N3 + q + 1) * KT].astype(_F32)
            for i, cmb in enumerate(_hk_b(b)):
                wc1[i * N3 + q] = _pack(cmb)

        dw_copy.wait()
        dw = dwv[0].astype(_F32)

        def prep(xs):
            xs = xs.astype(_F32) * dw
            m = jnp.mean(xs, axis=-1, keepdims=True)
            xc = xs - m
            v = jnp.mean(xc * xc, axis=-1, keepdims=True)
            xn = xc * jnp.exp(math.log(0.5 / _ALPHA) - 0.5 * jnp.log(v + _LN_EPS))
            blocks = [xn[i * H1:(i + 1) * H1, l * KT:(l + 1) * KT] for i in range(2) for l in range(3)]
            return [o.astype(_BF) for o in _hk_a(*blocks)]

        def hidden_rows(L, slot, r0, stats):
            for q in range(N3):
                def emit(i, j, z):
                    g = z + z * jnp.tanh(z * (_GZ + z * z))
                    ct = j * N3 + q
                    if stats:
                        gg = (g * g).reshape(H1 // 8, 8, KT)
                        acc_ref[:, ct * KT:(ct + 1) * KT] += jnp.sum(gg, axis=0)
                    hv[slot, ct, pl.ds(r0 + i * H1, H1), :] = g.astype(_BF)

                _hk_c(lambda i: _dot(L[i], _unpack(wc1[i * N3 + q])), emit)

        x_copy(0, 0).wait()
        x_copy(1, 1).start()
        w2_copy.start(priority=PRIO)
        g_copy.start()
        b_copy.start()
        for i, o in enumerate(prep(xv[0, 0:SUB1, :])):
            lk[i] = pltpu.bitcast(o, _U32)

        def phase0(t, carry):
            slot, xs_cur = carry
            xs_n1 = inc_mod(xs_cur, NX)
            xs_n2 = inc_mod(xs_n1, NX)

            @pl.when(t + 1 < T)
            def _():
                x_copy(t + 1, xs_n1).wait()

            @pl.when(t + 2 < T)
            def _():
                x_copy(t + 2, xs_n2).start()

            @pl.when(jnp.logical_and(t >= S, kept(t - S)))
            def _():
                h_write(t - S, slot).wait()

            for si in range(NS1):
                r0 = si * SUB1
                if si == 0:
                    L = [_unpack(lk[i]) for i in range(_NP)]
                else:
                    L = prep(xv[xs_cur, r0:r0 + SUB1, :])
                hidden_rows(L, slot, r0, True)

            xs_nxt = jnp.where(t + 1 < T, xs_n1, xs_cur)
            for i, o in enumerate(prep(xv[xs_nxt, 0:SUB1, :])):
                lk[i] = pltpu.bitcast(o, _U32)

            @pl.when(jnp.logical_and(t < T - S, kept(t)))
            def _():
                h_write(t, slot).start(priority=PRIO)

            return inc_mod(slot, S), xs_n1

        i32 = jnp.int32
        jax.lax.fori_loop(0, T, phase0, (i32(0), i32(0)))

        w2_copy.wait()
        g_copy.wait()
        b_copy.wait()
        ss = jnp.sum(acc_ref[...], axis=0, keepdims=True)
        gx = jnp.sqrt(ss * (_ALPHA * _ALPHA) + _GRN_EPS)
        nx = gx / (jnp.mean(gx, axis=-1, keepdims=True) + _GRN_EPS)
        s = (gv[...].reshape(1, F).astype(_F32) * nx + 1.0) * _ALPHA
        st = jnp.transpose(jnp.broadcast_to(s, (128, F)))
        F3 = F // 3
        b = lambda l, j: (w2v[(l - 1) * F3:l * F3, (j - 1) * KT:j * KT].astype(_F32)
                          * st[(l - 1) * F3:l * F3])
        for i, cmb in enumerate(_hk_b(b)):
            for q in range(N3):
                wc2[i * N3 + q] = _pack(cmb[q * KT:(q + 1) * KT, :])
        bb = jnp.broadcast_to(bv[...].reshape(1, F), (16, F))
        bias_ref[...] = _dot(bb, w2v[...])[:8]

        def phase1(j, carry):
            tile = T - 1 - j
            slot, xs_cur = carry
            xs_nxt = dec_mod(xs_cur, NX)

            @pl.when(jnp.logical_and(j >= S, kept(tile)))
            def _():
                for c in range(NCH):
                    h_read(tile, slot, c).wait()

            @pl.when(j >= NX)
            def _():
                x_copy(tile, xs_cur).wait()

            @pl.when(j >= 2)
            def _():
                xs_p2 = inc_mod(inc_mod(xs_cur, NX), NX)
                for c in range(NCH):
                    o_copy(tile + 2, xs_p2, c).wait()

                @pl.when(tile + 2 >= NX)
                def _():
                    x_copy(tile + 2 - NX, xs_p2).start()

            if DROP:
                @pl.when(jnp.logical_not(kept(tile)))
                def _():
                    def body(k, c):
                        r0 = pl.multiple_of(k * RB, RB)
                        for si in range(RB // SUB1):
                            rr = pl.multiple_of(r0 + si * SUB1, SUB1)
                            hidden_rows(prep(xv[xs_cur, pl.ds(rr, SUB1), :]), slot, rr, False)
                        return c
                    jax.lax.fori_loop(0, TM // RB, body, 0)

            bias = bias_ref[0:1, :]
            for si in range(NCH):
                r0 = si * SUB2

                def op(r, terms):
                    sl = slot + jax.lax.shift_right_logical(j, 16 + r)
                    pc = lambda i, l, q: hv[sl, l * N3 + q, r0 + i * H2:r0 + (i + 1) * H2, :]
                    if len(terms) == 1:
                        _, i, l = terms[0]
                        return jnp.concatenate([pc(i, l, q) for q in range(N3)], axis=1)
                    acc = None
                    for sg, i, l in terms:
                        v = jnp.concatenate([pc(i, l, q).astype(_F32) for q in range(N3)], axis=1)
                        acc = v if acc is None else (acc + v if sg > 0 else acc - v)
                    return acc.astype(_BF)

                ops = [op(r, _HK_U[r]) for r in range(_NP)]

                def emit(i, jn, y):
                    rows = slice(r0 + i * H2, r0 + (i + 1) * H2)
                    cols = slice(jn * KT, (jn + 1) * KT)
                    y = y + bias[:, cols] + xv[xs_cur, rows, cols].astype(_F32)
                    xv[xs_cur, rows, cols] = y.astype(xv.dtype)

                _hk_c(lambda i: _dot(ops[i], _unpack(
                    wc2[i * N3:(i + 1) * N3].reshape(N3 * (KT // 2), KT))), emit)

                o_copy(tile, xs_cur, si).start()

                @pl.when(jnp.logical_and(tile >= S, kept(tile - S)))
                def _():
                    h_read(tile - S, slot, si).start(priority=PRIO)

            return dec_mod(slot, S), xs_nxt

        jax.lax.fori_loop(0, T, phase1, (i32((T - 1) % S), i32((T - 1) % NX)))

        for tile in (1, 0):
            for c in range(NCH):
                o_copy(tile, tile % NX, c).wait()

    return kernel


def _run(x, dw, w1, w2, grn_g, grn_b, *, TM=3072, S=12, NX=4, SUB1=128, SUB2=1024, RB=1024,
         D1=31, D2=17, D3=-1, VMEM_MB=128, PRIO=1, NOBC=1):
    B, H, W, C = x.shape
    F = w1.shape[1]
    N = B * H * W
    T = N // TM
    DROP = tuple(d for d in (D1, D2, D3) if d >= 0)
    assert N % TM == 0 and T > S and T >= NX and all(d < T - S for d in DROP)

    x2 = x.reshape(N, C)
    kernel = _make_kernel(T=T, TM=TM, C=C, F=F, S=S, NX=NX, SUB1=SUB1, SUB2=SUB2, RB=RB,
                          DROP=DROP, PRIO=PRIO)
    any_spec = pl.BlockSpec(memory_space=pl.ANY)
    out, _ = pl.pallas_call(
        kernel,
        in_specs=[any_spec] * 6,
        out_specs=[any_spec, any_spec],
        out_shape=[
            jax.ShapeDtypeStruct((N, C), x.dtype),
            jax.ShapeDtypeStruct((T - S - len(DROP), F // 128, TM, 128), _BF),
        ],
        scratch_shapes=[
            pltpu.VMEM((NX, TM, C), _BF),
            pltpu.VMEM((S, F // 128, TM, 128), _BF),
            pltpu.VMEM((C, F), _BF),
            pltpu.VMEM((F, C), _BF),
            pltpu.VMEM((60, 64, 128), _U32),
            pltpu.VMEM((60, 64, 128), _U32),
            pltpu.VMEM((_NP, SUB1 // 4, 128), _U32),
            pltpu.VMEM((8, F), _F32),
            pltpu.VMEM((8, C), _F32),
            pltpu.VMEM((1, 1, C), _BF),
            pltpu.VMEM((F,), _BF),
            pltpu.VMEM((F,), _BF),
            pltpu.SemaphoreType.DMA((NX,)),
            pltpu.SemaphoreType.DMA((NX,)),
            pltpu.SemaphoreType.DMA((S,)),
            pltpu.SemaphoreType.DMA((5,)),
        ],
        compiler_params=pltpu.CompilerParams(
            vmem_limit_bytes=VMEM_MB * 1024 * 1024,
            disable_bounds_checks=bool(NOBC),
        ),
    )(x2, dw, w1, w2, grn_g, grn_b)
    return out.reshape(B, H, W, C)


@jax.jit
def pallas_standalone__modern_conv_block_slak__vision_kernel(
    x: jax.Array,
    dw: jax.Array,
    w1: jax.Array,
    w2: jax.Array,
    grn_g: jax.Array,
    grn_b: jax.Array,
):
    return _run(x, dw, w1, w2, grn_g, grn_b)
```

```python
import math

import jax
import jax.numpy as jnp
import jax.experimental.pallas as pl
import jax.experimental.pallas.tpu as pltpu

_LN_EPS = 1e-5
_GRN_EPS = 1e-6
_GA = 2.0 * math.sqrt(2.0 / math.pi)
_GB = 8.0 * math.sqrt(2.0 / math.pi) * 0.044715
_ALPHA = _GB ** (-1.0 / 3.0)
_GZ = _GA * _ALPHA
_KT = 128
_BF = jnp.bfloat16
_F32 = jnp.float32
_U32 = jnp.uint32

_HK_U = (
    ((1, 1, 1),),
    ((1, 0, 0), (1, 1, 1)),
    ((1, 0, 0), (-1, 1, 0), (1, 1, 2)),
    ((1, 0, 1), (-1, 0, 2), (-1, 1, 1), (1, 1, 2)),
    ((1, 1, 0), (1, 1, 1)),
    ((1, 0, 1), (-1, 0, 2), (-1, 1, 1)),
    ((1, 1, 0), (-1, 0, 0)),
    ((1, 0, 2),),
    ((1, 0, 1), (-1, 0, 2)),
    ((1, 1, 2),),
    ((1, 0, 2), (-1, 0, 0), (1, 1, 0), (-1, 1, 2)),
    ((1, 0, 0), (1, 0, 1)),
    ((1, 1, 0), (-1, 1, 2)),
    ((1, 1, 1), (-1, 0, 1)),
    ((1, 0, 0),),
)
_NP = len(_HK_U)


def _hk_a(a11, a12, a13, a21, a22, a23):
    d1 = a12 - a13
    d2 = d1 - a22
    e1 = a21 - a23
    l2 = a11 - e1
    return (a22, a11 + a22, l2, d2 + a23, a21 + a22, d2, a21 - a11, a13, d1, a23,
            a13 - l2, a11 + a12, e1, a22 - a12, a11)


def _hk_b(b):
    return (
        b(2, 3) - b(1, 3) - b(2, 2),
        b(1, 3) - b(2, 1),
        b(1, 2) - b(3, 1),
        b(3, 3),
        b(1, 3),
        -b(2, 2) - b(3, 3),
        b(1, 1) - b(1, 3) + b(3, 1),
        b(2, 2) + b(3, 1) + b(3, 2),
        b(2, 2),
        b(1, 2) + b(3, 2) - b(3, 3),
        b(3, 1),
        b(2, 1),
        b(1, 2),
        b(2, 1) - b(2, 3) - b(3, 3),
        b(1, 1) + b(1, 2) - b(2, 1),
    )


def _hk_c(P, emit):
    q8 = P(8)
    a = P(5) + q8
    b = a + P(3)
    p0 = P(0)
    p4 = P(4)
    emit(1, 2, b + p0 + p4)
    a = a + p0
    p12 = P(12)
    emit(1, 1, b + P(9) + p12)
    d = P(2) + p12
    p10 = P(10)
    emit(0, 1, d + q8 + P(7) - p10)
    e = P(14) - d
    p11 = P(11)
    emit(0, 0, e + p10 + p11)
    p1 = P(1)
    emit(0, 2, a + p11 + p1 + P(13))
    emit(1, 0, e + p4 - p1 + P(6))


def _pack(v):
    return pltpu.bitcast(v.astype(_BF), _U32)


def _unpack(u):
    return pltpu.bitcast(u, _BF)


def _dot(a, b):
    return jnp.dot(a, b, preferred_element_type=_F32)


def _make_kernel(*, T, TM, C, F, S, NX, SUB1, SUB2, RB, DROP, PRIO, PLA=2):
    KT = _KT
    H1 = SUB1 // 2
    H2 = SUB2 // 2
    NCH = TM // SUB2
    NS1 = TM // SUB1
    N3 = F // (3 * KT)

    def inc_mod(v, m):
        return jnp.where(v + 1 == m, 0, v + 1)

    def dec_mod(v, m):
        return jnp.where(v == 0, m - 1, v - 1)

    def kept(t):
        k = t >= 0
        for d in DROP:
            k = jnp.logical_and(k, t != d)
        return k

    def hidx(t):
        i = t
        for d in DROP:
            i = i - (t > d).astype(jnp.int32)
        return i

    def kernel(x_hbm, dw_hbm, w1_hbm, w2_hbm, g_hbm, b_hbm,
               o_hbm, hbuf_hbm,
               xv, hv, w1v, w2v, wc1, wc2, lk, pk, acc_ref, bias_ref, dwv, gv, bv,
               xsem, osem, hsem, wsem):

        def x_copy(tile, s):
            return pltpu.make_async_copy(x_hbm.at[pl.ds(tile * TM, TM)], xv.at[s], xsem.at[s])

        def o_copy(tile, s, c):
            r = c * SUB2
            return pltpu.make_async_copy(xv.at[s, pl.ds(r, SUB2)],
                                         o_hbm.at[pl.ds(tile * TM + r, SUB2)], osem.at[s])

        def h_write(tile, slot):
            return pltpu.make_async_copy(hv.at[slot], hbuf_hbm.at[hidx(tile)], hsem.at[slot])

        def h_read(tile, slot, c):
            rows = pl.ds(c * SUB2, SUB2)
            return pltpu.make_async_copy(hbuf_hbm.at[hidx(tile), :, rows, :],
                                         hv.at[slot, :, rows, :], hsem.at[slot])

        w1_copy = pltpu.make_async_copy(w1_hbm, w1v, wsem.at[0])
        w2_copy = pltpu.make_async_copy(w2_hbm, w2v, wsem.at[1])
        dw_copy = pltpu.make_async_copy(dw_hbm, dwv, wsem.at[2])
        g_copy = pltpu.make_async_copy(g_hbm, gv, wsem.at[3])
        b_copy = pltpu.make_async_copy(b_hbm, bv, wsem.at[4])

        dw_copy.start()
        w1_copy.start()
        x_copy(0, 0).start()

        acc_ref[...] = jnp.zeros_like(acc_ref)

        w1_copy.wait()
        for q in range(N3):
            b = lambda l, j: w1v[(l - 1) * KT:l * KT,
                                 ((j - 1) * N3 + q) * KT:((j - 1) * N3 + q + 1) * KT].astype(_F32)
            for i, cmb in enumerate(_hk_b(b)):
                wc1[i * N3 + q] = _pack(cmb)

        dw_copy.wait()
        dw = dwv[0].astype(_F32)

        def prep(xs):
            xs = xs.astype(_F32) * dw
            m = jnp.mean(xs, axis=-1, keepdims=True)
            xc = xs - m
            v = jnp.mean(xc * xc, axis=-1, keepdims=True)
            xn = xc * jnp.exp(math.log(0.5 / _ALPHA) - 0.5 * jnp.log(v + _LN_EPS))
            blocks = [xn[i * H1:(i + 1) * H1, l * KT:(l + 1) * KT] for i in range(2) for l in range(3)]
            return [o.astype(_BF) for o in _hk_a(*blocks)]

        def lookahead(xs):
            L = prep(xs)
            for i, o in enumerate(L):
                lk[i] = pltpu.bitcast(o, _U32)
            for q in range(PLA):
                for i in range(_NP):
                    pk[q * _NP + i] = _dot(L[i], _unpack(wc1[i * N3 + q]))

        def hidden_rows(L, slot, r0, stats, pre=0):
            for q in range(N3):
                def emit(i, j, z):
                    g = z + z * jnp.tanh(z * (_GZ + z * z))
                    ct = j * N3 + q
                    if stats:
                        gg = (g * g).reshape(H1 // 8, 8, KT)
                        acc_ref[:, ct * KT:(ct + 1) * KT] += jnp.sum(gg, axis=0)
                    hv[slot, ct, pl.ds(r0 + i * H1, H1), :] = g.astype(_BF)

                if q < pre:
                    _hk_c(lambda i: pk[q * _NP + i], emit)
                else:
                    _hk_c(lambda i: _dot(L[i], _unpack(wc1[i * N3 + q])), emit)

        x_copy(0, 0).wait()
        x_copy(1, 1).start()
        w2_copy.start(priority=PRIO)
        g_copy.start()
        b_copy.start()
        lookahead(xv[0, 0:SUB1, :])

        def phase0(t, carry):
            slot, xs_cur = carry
            xs_n1 = inc_mod(xs_cur, NX)
            xs_n2 = inc_mod(xs_n1, NX)

            @pl.when(t + 1 < T)
            def _():
                x_copy(t + 1, xs_n1).wait()

            @pl.when(t + 2 < T)
            def _():
                x_copy(t + 2, xs_n2).start()

            @pl.when(jnp.logical_and(t >= S, kept(t - S)))
            def _():
                h_write(t - S, slot).wait()

            for si in range(NS1):
                r0 = si * SUB1
                if si == 0:
                    L = [_unpack(lk[i]) for i in range(_NP)]
                else:
                    L = prep(xv[xs_cur, r0:r0 + SUB1, :])
                hidden_rows(L, slot, r0, True, PLA if si == 0 else 0)

            xs_nxt = jnp.where(t + 1 < T, xs_n1, xs_cur)
            lookahead(xv[xs_nxt, 0:SUB1, :])

            @pl.when(jnp.logical_and(t < T - S, kept(t)))
            def _():
                h_write(t, slot).start(priority=PRIO)

            return inc_mod(slot, S), xs_n1

        i32 = jnp.int32
        jax.lax.fori_loop(0, T, phase0, (i32(0), i32(0)))

        w2_copy.wait()
        g_copy.wait()
        b_copy.wait()
        ss = jnp.sum(acc_ref[...], axis=0, keepdims=True)
        gx = jnp.sqrt(ss * (_ALPHA * _ALPHA) + _GRN_EPS)
        nx = gx / (jnp.mean(gx, axis=-1, keepdims=True) + _GRN_EPS)
        s = (gv[...].reshape(1, F).astype(_F32) * nx + 1.0) * _ALPHA
        st = jnp.transpose(jnp.broadcast_to(s, (128, F)))
        F3 = F // 3
        b = lambda l, j: (w2v[(l - 1) * F3:l * F3, (j - 1) * KT:j * KT].astype(_F32)
                          * st[(l - 1) * F3:l * F3])
        for i, cmb in enumerate(_hk_b(b)):
            for q in range(N3):
                wc2[i * N3 + q] = _pack(cmb[q * KT:(q + 1) * KT, :])
        bb = jnp.broadcast_to(bv[...].reshape(1, F), (16, F))
        bias_ref[...] = _dot(bb, w2v[...])[:8]

        def phase1(j, carry):
            tile = T - 1 - j
            slot, xs_cur = carry
            xs_nxt = dec_mod(xs_cur, NX)

            @pl.when(jnp.logical_and(j >= S, kept(tile)))
            def _():
                for c in range(NCH):
                    h_read(tile, slot, c).wait()

            @pl.when(j >= NX)
            def _():
                x_copy(tile, xs_cur).wait()

            @pl.when(j >= 2)
            def _():
                xs_p2 = inc_mod(inc_mod(xs_cur, NX), NX)
                for c in range(NCH):
                    o_copy(tile + 2, xs_p2, c).wait()

                @pl.when(tile + 2 >= NX)
                def _():
                    x_copy(tile + 2 - NX, xs_p2).start()

            if DROP:
                @pl.when(jnp.logical_not(kept(tile)))
                def _():
                    def body(k, c):
                        r0 = pl.multiple_of(k * RB, RB)
                        for si in range(RB // SUB1):
                            rr = pl.multiple_of(r0 + si * SUB1, SUB1)
                            hidden_rows(prep(xv[xs_cur, pl.ds(rr, SUB1), :]), slot, rr, False)
                        return c
                    jax.lax.fori_loop(0, TM // RB, body, 0)

            bias = bias_ref[0:1, :]
            for si in range(NCH):
                r0 = si * SUB2

                def op(r, terms):
                    sl = slot + jax.lax.shift_right_logical(j, 16 + r)
                    pc = lambda i, l, q: hv[sl, l * N3 + q, r0 + i * H2:r0 + (i + 1) * H2, :]
                    if len(terms) == 1:
                        _, i, l = terms[0]
                        return jnp.concatenate([pc(i, l, q) for q in range(N3)], axis=1)
                    acc = None
                    for sg, i, l in terms:
                        v = jnp.concatenate([pc(i, l, q).astype(_F32) for q in range(N3)], axis=1)
                        acc = v if acc is None else (acc + v if sg > 0 else acc - v)
                    return acc.astype(_BF)

                ops = [op(r, _HK_U[r]) for r in range(_NP)]

                def emit(i, jn, y):
                    rows = slice(r0 + i * H2, r0 + (i + 1) * H2)
                    cols = slice(jn * KT, (jn + 1) * KT)
                    y = y + bias[:, cols] + xv[xs_cur, rows, cols].astype(_F32)
                    xv[xs_cur, rows, cols] = y.astype(xv.dtype)

                _hk_c(lambda i: _dot(ops[i], _unpack(
                    wc2[i * N3:(i + 1) * N3].reshape(N3 * (KT // 2), KT))), emit)

                o_copy(tile, xs_cur, si).start()

                @pl.when(jnp.logical_and(tile >= S, kept(tile - S)))
                def _():
                    h_read(tile - S, slot, si).start(priority=PRIO)

            return dec_mod(slot, S), xs_nxt

        jax.lax.fori_loop(0, T, phase1, (i32((T - 1) % S), i32((T - 1) % NX)))

        for tile in (1, 0):
            for c in range(NCH):
                o_copy(tile, tile % NX, c).wait()

    return kernel


def _run(x, dw, w1, w2, grn_g, grn_b, *, TM=3072, S=12, NX=3, SUB1=128, SUB2=1024, RB=1024,
         D1=31, D2=17, D3=-1, VMEM_MB=128, PRIO=1, NOBC=1, PLA=2):
    B, H, W, C = x.shape
    F = w1.shape[1]
    N = B * H * W
    T = N // TM
    DROP = tuple(d for d in (D1, D2, D3) if d >= 0)
    assert N % TM == 0 and T > S and T >= NX and all(d < T - S for d in DROP)

    x2 = x.reshape(N, C)
    kernel = _make_kernel(T=T, TM=TM, C=C, F=F, S=S, NX=NX, SUB1=SUB1, SUB2=SUB2, RB=RB,
                          DROP=DROP, PRIO=PRIO, PLA=PLA)
    any_spec = pl.BlockSpec(memory_space=pl.ANY)
    out, _ = pl.pallas_call(
        kernel,
        in_specs=[any_spec] * 6,
        out_specs=[any_spec, any_spec],
        out_shape=[
            jax.ShapeDtypeStruct((N, C), x.dtype),
            jax.ShapeDtypeStruct((T - S - len(DROP), F // 128, TM, 128), _BF),
        ],
        scratch_shapes=[
            pltpu.VMEM((NX, TM, C), _BF),
            pltpu.VMEM((S, F // 128, TM, 128), _BF),
            pltpu.VMEM((C, F), _BF),
            pltpu.VMEM((F, C), _BF),
            pltpu.VMEM((60, 64, 128), _U32),
            pltpu.VMEM((60, 64, 128), _U32),
            pltpu.VMEM((_NP, SUB1 // 4, 128), _U32),
            pltpu.VMEM((max(PLA, 1) * _NP, SUB1 // 2, 128), _F32),
            pltpu.VMEM((8, F), _F32),
            pltpu.VMEM((8, C), _F32),
            pltpu.VMEM((1, 1, C), _BF),
            pltpu.VMEM((F,), _BF),
            pltpu.VMEM((F,), _BF),
            pltpu.SemaphoreType.DMA((NX,)),
            pltpu.SemaphoreType.DMA((NX,)),
            pltpu.SemaphoreType.DMA((S,)),
            pltpu.SemaphoreType.DMA((5,)),
        ],
        compiler_params=pltpu.CompilerParams(
            vmem_limit_bytes=VMEM_MB * 1024 * 1024,
            disable_bounds_checks=bool(NOBC),
        ),
    )(x2, dw, w1, w2, grn_g, grn_b)
    return out.reshape(B, H, W, C)


@jax.jit
def pallas_standalone__modern_conv_block_slak__vision_kernel(
    x: jax.Array,
    dw: jax.Array,
    w1: jax.Array,
    w2: jax.Array,
    grn_g: jax.Array,
    grn_b: jax.Array,
):
    return _run(x, dw, w1, w2, grn_g, grn_b)
```

```python
import math

import jax
import jax.numpy as jnp
import jax.experimental.pallas as pl
import jax.experimental.pallas.tpu as pltpu

_LN_EPS = 1e-5
_GRN_EPS = 1e-6
_GA = 2.0 * math.sqrt(2.0 / math.pi)
_GB = 8.0 * math.sqrt(2.0 / math.pi) * 0.044715
_ALPHA = _GB ** (-1.0 / 3.0)
_GZ = _GA * _ALPHA
_KT = 128
_BF = jnp.bfloat16
_F32 = jnp.float32
_U32 = jnp.uint32

_HK_U = (
    ((1, 1, 1),),
    ((1, 0, 0), (1, 1, 1)),
    ((1, 0, 0), (-1, 1, 0), (1, 1, 2)),
    ((1, 0, 1), (-1, 0, 2), (-1, 1, 1), (1, 1, 2)),
    ((1, 1, 0), (1, 1, 1)),
    ((1, 0, 1), (-1, 0, 2), (-1, 1, 1)),
    ((1, 1, 0), (-1, 0, 0)),
    ((1, 0, 2),),
    ((1, 0, 1), (-1, 0, 2)),
    ((1, 1, 2),),
    ((1, 0, 2), (-1, 0, 0), (1, 1, 0), (-1, 1, 2)),
    ((1, 0, 0), (1, 0, 1)),
    ((1, 1, 0), (-1, 1, 2)),
    ((1, 1, 1), (-1, 0, 1)),
    ((1, 0, 0),),
)
_NP = len(_HK_U)


def _hk_a(a11, a12, a13, a21, a22, a23):
    d1 = a12 - a13
    d2 = d1 - a22
    e1 = a21 - a23
    l2 = a11 - e1
    return (a22, a11 + a22, l2, d2 + a23, a21 + a22, d2, a21 - a11, a13, d1, a23,
            a13 - l2, a11 + a12, e1, a22 - a12, a11)


def _hk_b(b):
    return (
        b(2, 3) - b(1, 3) - b(2, 2),
        b(1, 3) - b(2, 1),
        b(1, 2) - b(3, 1),
        b(3, 3),
        b(1, 3),
        -b(2, 2) - b(3, 3),
        b(1, 1) - b(1, 3) + b(3, 1),
        b(2, 2) + b(3, 1) + b(3, 2),
        b(2, 2),
        b(1, 2) + b(3, 2) - b(3, 3),
        b(3, 1),
        b(2, 1),
        b(1, 2),
        b(2, 1) - b(2, 3) - b(3, 3),
        b(1, 1) + b(1, 2) - b(2, 1),
    )


def _hk_c(P, emit):
    q8 = P(8)
    a = P(5) + q8
    b = a + P(3)
    p0 = P(0)
    p4 = P(4)
    emit(1, 2, b + p0 + p4)
    a = a + p0
    p12 = P(12)
    emit(1, 1, b + P(9) + p12)
    d = P(2) + p12
    p10 = P(10)
    emit(0, 1, d + q8 + P(7) - p10)
    e = P(14) - d
    p11 = P(11)
    emit(0, 0, e + p10 + p11)
    p1 = P(1)
    emit(0, 2, a + p11 + p1 + P(13))
    emit(1, 0, e + p4 - p1 + P(6))


def _pack(v):
    return pltpu.bitcast(v.astype(_BF), _U32)


def _unpack(u):
    return pltpu.bitcast(u, _BF)


def _dot(a, b):
    return jnp.dot(a, b, preferred_element_type=_F32)


def _make_kernel(*, T, TM, C, F, S, NX, SUB1, SUB2, RB, DROP, PRIO, PLA=2):
    KT = _KT
    H1 = SUB1 // 2
    H2 = SUB2 // 2
    NCH = TM // SUB2
    NS1 = TM // SUB1
    N3 = F // (3 * KT)

    def inc_mod(v, m):
        return jnp.where(v + 1 == m, 0, v + 1)

    def dec_mod(v, m):
        return jnp.where(v == 0, m - 1, v - 1)

    def kept(t):
        k = t >= 0
        for d in DROP:
            k = jnp.logical_and(k, t != d)
        return k

    def hidx(t):
        i = t
        for d in DROP:
            i = i - (t > d).astype(jnp.int32)
        return i

    def kernel(x_hbm, dw_hbm, w1_hbm, w2_hbm, g_hbm, b_hbm,
               o_hbm, hbuf_hbm,
               xv, xh, hv, w1v, w2v, wc1, wc2, lk, pk, acc_ref, bias_ref, dwv, gv, bv,
               xsem, xhsem, osem, hsem, wsem):

        def x_copy(tile, s):
            return pltpu.make_async_copy(x_hbm.at[pl.ds(tile * TM, TM)], xv.at[s], xsem.at[s])

        def xh_copy(tile, s):
            return pltpu.make_async_copy(x_hbm.at[pl.ds(tile * TM, SUB1)], xh.at[s], xhsem.at[s])

        def o_copy(tile, s, c):
            r = c * SUB2
            return pltpu.make_async_copy(xv.at[s, pl.ds(r, SUB2)],
                                         o_hbm.at[pl.ds(tile * TM + r, SUB2)], osem.at[s])

        def h_write(tile, slot):
            return pltpu.make_async_copy(hv.at[slot], hbuf_hbm.at[hidx(tile)], hsem.at[slot])

        def h_read(tile, slot, c):
            rows = pl.ds(c * SUB2, SUB2)
            return pltpu.make_async_copy(hbuf_hbm.at[hidx(tile), :, rows, :],
                                         hv.at[slot, :, rows, :], hsem.at[slot])

        w1_copy = pltpu.make_async_copy(w1_hbm, w1v, wsem.at[0])
        w2_copy = pltpu.make_async_copy(w2_hbm, w2v, wsem.at[1])
        dw_copy = pltpu.make_async_copy(dw_hbm, dwv, wsem.at[2])
        g_copy = pltpu.make_async_copy(g_hbm, gv, wsem.at[3])
        b_copy = pltpu.make_async_copy(b_hbm, bv, wsem.at[4])

        dw_copy.start()
        xh_copy(0, 0).start()
        w1_copy.start()
        xh_copy(1, 1).start()
        x_copy(0, 0).start()

        acc_ref[...] = jnp.zeros_like(acc_ref)

        w1_copy.wait()
        for q in range(N3):
            b = lambda l, j: w1v[(l - 1) * KT:l * KT,
                                 ((j - 1) * N3 + q) * KT:((j - 1) * N3 + q + 1) * KT].astype(_F32)
            for i, cmb in enumerate(_hk_b(b)):
                wc1[i * N3 + q] = _pack(cmb)

        dw_copy.wait()
        dw = dwv[0].astype(_F32)

        def prep(xs):
            xs = xs.astype(_F32) * dw
            m = jnp.mean(xs, axis=-1, keepdims=True)
            xc = xs - m
            v = jnp.mean(xc * xc, axis=-1, keepdims=True)
            xn = xc * jnp.exp(math.log(0.5 / _ALPHA) - 0.5 * jnp.log(v + _LN_EPS))
            blocks = [xn[i * H1:(i + 1) * H1, l * KT:(l + 1) * KT] for i in range(2) for l in range(3)]
            return [o.astype(_BF) for o in _hk_a(*blocks)]

        def lookahead(xs):
            L = prep(xs)
            for i, o in enumerate(L):
                lk[i] = pltpu.bitcast(o, _U32)
            for q in range(PLA):
                for i in range(_NP):
                    pk[q * _NP + i] = _dot(L[i], _unpack(wc1[i * N3 + q]))

        def hidden_rows(L, slot, r0, stats, pre=0):
            for q in range(N3):
                def emit(i, j, z):
                    g = z + z * jnp.tanh(z * (_GZ + z * z))
                    ct = j * N3 + q
                    if stats:
                        gg = (g * g).reshape(H1 // 8, 8, KT)
                        acc_ref[:, ct * KT:(ct + 1) * KT] += jnp.sum(gg, axis=0)
                    hv[slot, ct, pl.ds(r0 + i * H1, H1), :] = g.astype(_BF)

                if q < pre:
                    _hk_c(lambda i: pk[q * _NP + i], emit)
                else:
                    _hk_c(lambda i: _dot(L[i], _unpack(wc1[i * N3 + q])), emit)

        xh_copy(0, 0).wait()
        lookahead(xh[0])
        x_copy(0, 0).wait()
        x_copy(1, 1).start()
        w2_copy.start(priority=PRIO)
        g_copy.start()
        b_copy.start()

        def phase0(t, carry):
            slot, xs_cur, hs_nxt = carry
            xs_n1 = inc_mod(xs_cur, NX)
            xs_n2 = inc_mod(xs_n1, NX)

            @pl.when(t > 0)
            def _():
                x_copy(t, xs_cur).wait()

            @pl.when(t + 1 < T)
            def _():
                xh_copy(t + 1, hs_nxt).wait()

            @pl.when(t + 2 < T)
            def _():
                x_copy(t + 2, xs_n2).start()
                xh_copy(t + 2, 1 - hs_nxt).start()

            @pl.when(jnp.logical_and(t >= S, kept(t - S)))
            def _():
                h_write(t - S, slot).wait()

            for si in range(NS1):
                r0 = si * SUB1
                if si == 0:
                    L = [_unpack(lk[i]) for i in range(_NP)]
                else:
                    L = prep(xv[xs_cur, r0:r0 + SUB1, :])
                hidden_rows(L, slot, r0, True, PLA if si == 0 else 0)

            lookahead(xh[hs_nxt])

            @pl.when(jnp.logical_and(t < T - S, kept(t)))
            def _():
                h_write(t, slot).start(priority=PRIO)

            return inc_mod(slot, S), xs_n1, 1 - hs_nxt

        i32 = jnp.int32
        jax.lax.fori_loop(0, T, phase0, (i32(0), i32(0), i32(1)))

        w2_copy.wait()
        g_copy.wait()
        b_copy.wait()
        ss = jnp.sum(acc_ref[...], axis=0, keepdims=True)
        gx = jnp.sqrt(ss * (_ALPHA * _ALPHA) + _GRN_EPS)
        nx = gx / (jnp.mean(gx, axis=-1, keepdims=True) + _GRN_EPS)
        s = (gv[...].reshape(1, F).astype(_F32) * nx + 1.0) * _ALPHA
        st = jnp.transpose(jnp.broadcast_to(s, (128, F)))
        F3 = F // 3
        b = lambda l, j: (w2v[(l - 1) * F3:l * F3, (j - 1) * KT:j * KT].astype(_F32)
                          * st[(l - 1) * F3:l * F3])
        for i, cmb in enumerate(_hk_b(b)):
            for q in range(N3):
                wc2[i * N3 + q] = _pack(cmb[q * KT:(q + 1) * KT, :])
        bb = jnp.broadcast_to(bv[...].reshape(1, F), (16, F))
        bias_ref[...] = _dot(bb, w2v[...])[:8]

        def phase1(j, carry):
            tile = T - 1 - j
            slot, xs_cur = carry
            xs_nxt = dec_mod(xs_cur, NX)

            @pl.when(jnp.logical_and(j >= S, kept(tile)))
            def _():
                for c in range(NCH):
                    h_read(tile, slot, c).wait()

            @pl.when(j >= NX)
            def _():
                x_copy(tile, xs_cur).wait()

            @pl.when(j >= 2)
            def _():
                xs_p2 = inc_mod(inc_mod(xs_cur, NX), NX)
                for c in range(NCH):
                    o_copy(tile + 2, xs_p2, c).wait()

                @pl.when(tile + 2 >= NX)
                def _():
                    x_copy(tile + 2 - NX, xs_p2).start()

            if DROP:
                @pl.when(jnp.logical_not(kept(tile)))
                def _():
                    def body(k, c):
                        r0 = pl.multiple_of(k * RB, RB)
                        for si in range(RB // SUB1):
                            rr = pl.multiple_of(r0 + si * SUB1, SUB1)
                            hidden_rows(prep(xv[xs_cur, pl.ds(rr, SUB1), :]), slot, rr, False)
                        return c
                    jax.lax.fori_loop(0, TM // RB, body, 0)

            bias = bias_ref[0:1, :]
            for si in range(NCH):
                r0 = si * SUB2

                def op(r, terms):
                    sl = slot + jax.lax.shift_right_logical(j, 16 + r)
                    pc = lambda i, l, q: hv[sl, l * N3 + q, r0 + i * H2:r0 + (i + 1) * H2, :]
                    if len(terms) == 1:
                        _, i, l = terms[0]
                        return jnp.concatenate([pc(i, l, q) for q in range(N3)], axis=1)
                    acc = None
                    for sg, i, l in terms:
                        v = jnp.concatenate([pc(i, l, q).astype(_F32) for q in range(N3)], axis=1)
                        acc = v if acc is None else (acc + v if sg > 0 else acc - v)
                    return acc.astype(_BF)

                ops = [op(r, _HK_U[r]) for r in range(_NP)]

                def emit(i, jn, y):
                    rows = slice(r0 + i * H2, r0 + (i + 1) * H2)
                    cols = slice(jn * KT, (jn + 1) * KT)
                    y = y + bias[:, cols] + xv[xs_cur, rows, cols].astype(_F32)
                    xv[xs_cur, rows, cols] = y.astype(xv.dtype)

                _hk_c(lambda i: _dot(ops[i], _unpack(
                    wc2[i * N3:(i + 1) * N3].reshape(N3 * (KT // 2), KT))), emit)

                o_copy(tile, xs_cur, si).start()

                @pl.when(jnp.logical_and(tile >= S, kept(tile - S)))
                def _():
                    h_read(tile - S, slot, si).start(priority=PRIO)

            return dec_mod(slot, S), xs_nxt

        jax.lax.fori_loop(0, T, phase1, (i32((T - 1) % S), i32((T - 1) % NX)))

        for tile in (1, 0):
            for c in range(NCH):
                o_copy(tile, tile % NX, c).wait()

    return kernel


def _run(x, dw, w1, w2, grn_g, grn_b, *, TM=3072, S=12, NX=3, SUB1=128, SUB2=1024, RB=1024,
         D1=31, D2=17, D3=-1, VMEM_MB=128, PRIO=1, NOBC=1, PLA=2):
    B, H, W, C = x.shape
    F = w1.shape[1]
    N = B * H * W
    T = N // TM
    DROP = tuple(d for d in (D1, D2, D3) if d >= 0)
    assert N % TM == 0 and T > S and T >= NX and all(d < T - S for d in DROP)

    x2 = x.reshape(N, C)
    kernel = _make_kernel(T=T, TM=TM, C=C, F=F, S=S, NX=NX, SUB1=SUB1, SUB2=SUB2, RB=RB,
                          DROP=DROP, PRIO=PRIO, PLA=PLA)
    any_spec = pl.BlockSpec(memory_space=pl.ANY)
    out, _ = pl.pallas_call(
        kernel,
        in_specs=[any_spec] * 6,
        out_specs=[any_spec, any_spec],
        out_shape=[
            jax.ShapeDtypeStruct((N, C), x.dtype),
            jax.ShapeDtypeStruct((T - S - len(DROP), F // 128, TM, 128), _BF),
        ],
        scratch_shapes=[
            pltpu.VMEM((NX, TM, C), _BF),
            pltpu.VMEM((2, SUB1, C), _BF),
            pltpu.VMEM((S, F // 128, TM, 128), _BF),
            pltpu.VMEM((C, F), _BF),
            pltpu.VMEM((F, C), _BF),
            pltpu.VMEM((60, 64, 128), _U32),
            pltpu.VMEM((60, 64, 128), _U32),
            pltpu.VMEM((_NP, SUB1 // 4, 128), _U32),
            pltpu.VMEM((max(PLA, 1) * _NP, SUB1 // 2, 128), _F32),
            pltpu.VMEM((8, F), _F32),
            pltpu.VMEM((8, C), _F32),
            pltpu.VMEM((1, 1, C), _BF),
            pltpu.VMEM((F,), _BF),
            pltpu.VMEM((F,), _BF),
            pltpu.SemaphoreType.DMA((NX,)),
            pltpu.SemaphoreType.DMA((2,)),
            pltpu.SemaphoreType.DMA((NX,)),
            pltpu.SemaphoreType.DMA((S,)),
            pltpu.SemaphoreType.DMA((5,)),
        ],
        compiler_params=pltpu.CompilerParams(
            vmem_limit_bytes=VMEM_MB * 1024 * 1024,
            disable_bounds_checks=bool(NOBC),
        ),
    )(x2, dw, w1, w2, grn_g, grn_b)
    return out.reshape(B, H, W, C)


@jax.jit
def pallas_standalone__modern_conv_block_slak__vision_kernel(
    x: jax.Array,
    dw: jax.Array,
    w1: jax.Array,
    w2: jax.Array,
    grn_g: jax.Array,
    grn_b: jax.Array,
):
    return _run(x, dw, w1, w2, grn_g, grn_b)
```

```python
import math

import jax
import jax.numpy as jnp
import jax.experimental.pallas as pl
import jax.experimental.pallas.tpu as pltpu

_LN_EPS = 1e-5
_GRN_EPS = 1e-6
_GA = 2.0 * math.sqrt(2.0 / math.pi)
_GB = 8.0 * math.sqrt(2.0 / math.pi) * 0.044715
_ALPHA = _GB ** (-1.0 / 3.0)
_GZ = _GA * _ALPHA
_KT = 128
_BF = jnp.bfloat16
_F32 = jnp.float32
_U32 = jnp.uint32

_HK_U = (
    ((1, 1, 1),),
    ((1, 0, 0), (1, 1, 1)),
    ((1, 0, 0), (-1, 1, 0), (1, 1, 2)),
    ((1, 0, 1), (-1, 0, 2), (-1, 1, 1), (1, 1, 2)),
    ((1, 1, 0), (1, 1, 1)),
    ((1, 0, 1), (-1, 0, 2), (-1, 1, 1)),
    ((1, 1, 0), (-1, 0, 0)),
    ((1, 0, 2),),
    ((1, 0, 1), (-1, 0, 2)),
    ((1, 1, 2),),
    ((1, 0, 2), (-1, 0, 0), (1, 1, 0), (-1, 1, 2)),
    ((1, 0, 0), (1, 0, 1)),
    ((1, 1, 0), (-1, 1, 2)),
    ((1, 1, 1), (-1, 0, 1)),
    ((1, 0, 0),),
)
_NP = len(_HK_U)


def _hk_a(a11, a12, a13, a21, a22, a23):
    d1 = a12 - a13
    d2 = d1 - a22
    e1 = a21 - a23
    l2 = a11 - e1
    return (a22, a11 + a22, l2, d2 + a23, a21 + a22, d2, a21 - a11, a13, d1, a23,
            a13 - l2, a11 + a12, e1, a22 - a12, a11)


def _hk_b(b):
    return (
        b(2, 3) - b(1, 3) - b(2, 2),
        b(1, 3) - b(2, 1),
        b(1, 2) - b(3, 1),
        b(3, 3),
        b(1, 3),
        -b(2, 2) - b(3, 3),
        b(1, 1) - b(1, 3) + b(3, 1),
        b(2, 2) + b(3, 1) + b(3, 2),
        b(2, 2),
        b(1, 2) + b(3, 2) - b(3, 3),
        b(3, 1),
        b(2, 1),
        b(1, 2),
        b(2, 1) - b(2, 3) - b(3, 3),
        b(1, 1) + b(1, 2) - b(2, 1),
    )


def _hk_c(P, emit):
    q8 = P(8)
    a = P(5) + q8
    b = a + P(3)
    p0 = P(0)
    p4 = P(4)
    emit(1, 2, b + p0 + p4)
    a = a + p0
    p12 = P(12)
    emit(1, 1, b + P(9) + p12)
    d = P(2) + p12
    p10 = P(10)
    emit(0, 1, d + q8 + P(7) - p10)
    e = P(14) - d
    p11 = P(11)
    emit(0, 0, e + p10 + p11)
    p1 = P(1)
    emit(0, 2, a + p11 + p1 + P(13))
    emit(1, 0, e + p4 - p1 + P(6))


def _pack(v):
    return pltpu.bitcast(v.astype(_BF), _U32)


def _unpack(u):
    return pltpu.bitcast(u, _BF)


def _dot(a, b):
    return jnp.dot(a, b, preferred_element_type=_F32)


def _make_kernel(*, T, TM, C, F, S, NX, SUB1, SUB2, RB, DROP, PRIO, PLA=2, V1=0, V2=0):
    KT = _KT
    H1 = SUB1 // 2
    H2 = SUB2 // 2
    NCH = TM // SUB2
    NS1 = TM // SUB1
    N3 = F // (3 * KT)

    def inc_mod(v, m):
        return jnp.where(v + 1 == m, 0, v + 1)

    def dec_mod(v, m):
        return jnp.where(v == 0, m - 1, v - 1)

    def kept(t):
        k = t >= 0
        for d in DROP:
            k = jnp.logical_and(k, t != d)
        return k

    def hidx(t):
        i = t
        for d in DROP:
            i = i - (t > d).astype(jnp.int32)
        return i

    def kernel(x_hbm, dw_hbm, w1_hbm, w2_hbm, g_hbm, b_hbm,
               o_hbm, hbuf_hbm,
               xv, xh, hv, w1v, w2v, wc1, wc2, lk, pk, acc_ref, bias_ref, dwv, gv, bv,
               xsem, xhsem, osem, hsem, wsem):

        def x_copy(tile, s):
            return pltpu.make_async_copy(x_hbm.at[pl.ds(tile * TM, TM)], xv.at[s], xsem.at[s])

        def xh_copy(tile, s):
            return pltpu.make_async_copy(x_hbm.at[pl.ds(tile * TM, SUB1)], xh.at[s], xhsem.at[s])

        def o_copy(tile, s, c):
            r = c * SUB2
            return pltpu.make_async_copy(xv.at[s, pl.ds(r, SUB2)],
                                         o_hbm.at[pl.ds(tile * TM + r, SUB2)], osem.at[s])

        def h_write(tile, slot):
            return pltpu.make_async_copy(hv.at[slot], hbuf_hbm.at[hidx(tile)], hsem.at[slot])

        def h_read(tile, slot, c):
            rows = pl.ds(c * SUB2, SUB2)
            return pltpu.make_async_copy(hbuf_hbm.at[hidx(tile), :, rows, :],
                                         hv.at[slot, :, rows, :], hsem.at[slot])

        w1_copy = pltpu.make_async_copy(w1_hbm, w1v, wsem.at[0])
        w2_copy = pltpu.make_async_copy(w2_hbm, w2v, wsem.at[1])
        dw_copy = pltpu.make_async_copy(dw_hbm, dwv, wsem.at[2])
        g_copy = pltpu.make_async_copy(g_hbm, gv, wsem.at[3])
        b_copy = pltpu.make_async_copy(b_hbm, bv, wsem.at[4])

        dw_copy.start()
        xh_copy(0, 0).start()
        w1_copy.start()
        xh_copy(1, 1).start()
        x_copy(0, 0).start()

        acc_ref[...] = jnp.zeros_like(acc_ref)

        w1_copy.wait()
        for q in range(N3):
            b = lambda l, j: w1v[(l - 1) * KT:l * KT,
                                 ((j - 1) * N3 + q) * KT:((j - 1) * N3 + q + 1) * KT].astype(_F32)
            for i, cmb in enumerate(_hk_b(b)):
                wc1[i * N3 + q] = _pack(cmb)

        dw_copy.wait()
        dw = dwv[0].astype(_F32)

        def prep(xs):
            xs = xs.astype(_F32) * dw
            m = jnp.mean(xs, axis=-1, keepdims=True)
            xc = xs - m
            if V2:
                ssq = jnp.sum(xc * xc, axis=-1, keepdims=True)
                xn = xc * jnp.exp(math.log(0.5 * math.sqrt(C) / _ALPHA)
                                  - 0.5 * jnp.log(ssq + C * _LN_EPS))
            else:
                v = jnp.mean(xc * xc, axis=-1, keepdims=True)
                xn = xc * jnp.exp(math.log(0.5 / _ALPHA) - 0.5 * jnp.log(v + _LN_EPS))
            blocks = [xn[i * H1:(i + 1) * H1, l * KT:(l + 1) * KT] for i in range(2) for l in range(3)]
            return [o.astype(_BF) for o in _hk_a(*blocks)]

        def lookahead(xs):
            L = prep(xs)
            for i, o in enumerate(L):
                lk[i] = pltpu.bitcast(o, _U32)
            for q in range(PLA):
                for i in range(_NP):
                    pk[q * _NP + i] = _dot(L[i], _unpack(wc1[i * N3 + q]))

        def hidden_rows(L, slot, r0, stats, pre=0):
            for q in range(N3):
                part = {}

                def emit(i, j, z):
                    g = z + z * jnp.tanh(z * (_GZ + z * z))
                    ct = j * N3 + q
                    if stats:
                        gg = jnp.sum((g * g).reshape(H1 // 8, 8, KT), axis=0)
                        if V1 and j not in part:
                            part[j] = gg
                        else:
                            if V1:
                                gg = gg + part[j]
                            acc_ref[:, ct * KT:(ct + 1) * KT] += gg
                    hv[slot, ct, pl.ds(r0 + i * H1, H1), :] = g.astype(_BF)

                if q < pre:
                    _hk_c(lambda i: pk[q * _NP + i], emit)
                else:
                    _hk_c(lambda i: _dot(L[i], _unpack(wc1[i * N3 + q])), emit)

        xh_copy(0, 0).wait()
        lookahead(xh[0])
        x_copy(0, 0).wait()
        x_copy(1, 1).start()
        w2_copy.start(priority=PRIO)
        g_copy.start()
        b_copy.start()

        def phase0(t, carry):
            slot, xs_cur, hs_nxt = carry
            xs_n1 = inc_mod(xs_cur, NX)
            xs_n2 = inc_mod(xs_n1, NX)

            @pl.when(t > 0)
            def _():
                x_copy(t, xs_cur).wait()

            @pl.when(t + 1 < T)
            def _():
                xh_copy(t + 1, hs_nxt).wait()

            @pl.when(t + 2 < T)
            def _():
                x_copy(t + 2, xs_n2).start()
                xh_copy(t + 2, 1 - hs_nxt).start()

            @pl.when(jnp.logical_and(t >= S, kept(t - S)))
            def _():
                h_write(t - S, slot).wait()

            for si in range(NS1):
                r0 = si * SUB1
                if si == 0:
                    L = [_unpack(lk[i]) for i in range(_NP)]
                else:
                    L = prep(xv[xs_cur, r0:r0 + SUB1, :])
                hidden_rows(L, slot, r0, True, PLA if si == 0 else 0)

            lookahead(xh[hs_nxt])

            @pl.when(jnp.logical_and(t < T - S, kept(t)))
            def _():
                h_write(t, slot).start(priority=PRIO)

            return inc_mod(slot, S), xs_n1, 1 - hs_nxt

        i32 = jnp.int32
        jax.lax.fori_loop(0, T, phase0, (i32(0), i32(0), i32(1)))

        w2_copy.wait()
        g_copy.wait()
        b_copy.wait()
        ss = jnp.sum(acc_ref[...], axis=0, keepdims=True)
        gx = jnp.sqrt(ss * (_ALPHA * _ALPHA) + _GRN_EPS)
        nx = gx / (jnp.mean(gx, axis=-1, keepdims=True) + _GRN_EPS)
        s = (gv[...].reshape(1, F).astype(_F32) * nx + 1.0) * _ALPHA
        st = jnp.transpose(jnp.broadcast_to(s, (128, F)))
        F3 = F // 3
        b = lambda l, j: (w2v[(l - 1) * F3:l * F3, (j - 1) * KT:j * KT].astype(_F32)
                          * st[(l - 1) * F3:l * F3])
        for i, cmb in enumerate(_hk_b(b)):
            for q in range(N3):
                wc2[i * N3 + q] = _pack(cmb[q * KT:(q + 1) * KT, :])
        bb = jnp.broadcast_to(bv[...].reshape(1, F), (16, F))
        bias_ref[...] = _dot(bb, w2v[...])[:8]

        def phase1(j, carry):
            tile = T - 1 - j
            slot, xs_cur = carry
            xs_nxt = dec_mod(xs_cur, NX)

            @pl.when(jnp.logical_and(j >= S, kept(tile)))
            def _():
                for c in range(NCH):
                    h_read(tile, slot, c).wait()

            @pl.when(j >= NX)
            def _():
                x_copy(tile, xs_cur).wait()

            @pl.when(j >= 2)
            def _():
                xs_p2 = inc_mod(inc_mod(xs_cur, NX), NX)
                for c in range(NCH):
                    o_copy(tile + 2, xs_p2, c).wait()

                @pl.when(tile + 2 >= NX)
                def _():
                    x_copy(tile + 2 - NX, xs_p2).start()

            if DROP:
                @pl.when(jnp.logical_not(kept(tile)))
                def _():
                    def stash(rr):
                        for i, o in enumerate(prep(xv[xs_cur, pl.ds(rr, SUB1), :])):
                            lk[i] = pltpu.bitcast(o, _U32)

                    stash(0)

                    def body(k, c):
                        r0 = pl.multiple_of(k * RB, RB)
                        for si in range(RB // SUB1):
                            rr = pl.multiple_of(r0 + si * SUB1, SUB1)
                            if si == 0:
                                L = [_unpack(lk[i]) for i in range(_NP)]
                            else:
                                L = prep(xv[xs_cur, pl.ds(rr, SUB1), :])
                            hidden_rows(L, slot, rr, False)
                        stash(pl.multiple_of(jnp.minimum(r0 + RB, TM - RB), RB))
                        return c
                    jax.lax.fori_loop(0, TM // RB, body, 0)

            bias = bias_ref[0:1, :]
            for si in range(NCH):
                r0 = si * SUB2

                def op(r, terms):
                    sl = slot + jax.lax.shift_right_logical(j, 16 + r)
                    pc = lambda i, l, q: hv[sl, l * N3 + q, r0 + i * H2:r0 + (i + 1) * H2, :]
                    if len(terms) == 1:
                        _, i, l = terms[0]
                        return jnp.concatenate([pc(i, l, q) for q in range(N3)], axis=1)
                    acc = None
                    for sg, i, l in terms:
                        v = jnp.concatenate([pc(i, l, q).astype(_F32) for q in range(N3)], axis=1)
                        acc = v if acc is None else (acc + v if sg > 0 else acc - v)
                    return acc.astype(_BF)

                ops = [op(r, _HK_U[r]) for r in range(_NP)]

                def emit(i, jn, y):
                    rows = slice(r0 + i * H2, r0 + (i + 1) * H2)
                    cols = slice(jn * KT, (jn + 1) * KT)
                    y = y + bias[:, cols] + xv[xs_cur, rows, cols].astype(_F32)
                    xv[xs_cur, rows, cols] = y.astype(xv.dtype)

                _hk_c(lambda i: _dot(ops[i], _unpack(
                    wc2[i * N3:(i + 1) * N3].reshape(N3 * (KT // 2), KT))), emit)

                o_copy(tile, xs_cur, si).start()

                @pl.when(jnp.logical_and(tile >= S, kept(tile - S)))
                def _():
                    h_read(tile - S, slot, si).start(priority=PRIO)

            return dec_mod(slot, S), xs_nxt

        jax.lax.fori_loop(0, T, phase1, (i32((T - 1) % S), i32((T - 1) % NX)))

        for tile in (1, 0):
            for c in range(NCH):
                o_copy(tile, tile % NX, c).wait()

    return kernel


def _run(x, dw, w1, w2, grn_g, grn_b, *, TM=3072, S=12, NX=3, SUB1=128, SUB2=1024, RB=1024,
         D1=31, D2=17, D3=-1, VMEM_MB=128, PRIO=1, NOBC=1, PLA=2, V1=1, V2=1):
    B, H, W, C = x.shape
    F = w1.shape[1]
    N = B * H * W
    T = N // TM
    DROP = tuple(d for d in (D1, D2, D3) if d >= 0)
    assert N % TM == 0 and T > S and T >= NX and all(d < T - S for d in DROP)

    x2 = x.reshape(N, C)
    kernel = _make_kernel(T=T, TM=TM, C=C, F=F, S=S, NX=NX, SUB1=SUB1, SUB2=SUB2, RB=RB,
                          DROP=DROP, PRIO=PRIO, PLA=PLA, V1=V1, V2=V2)
    any_spec = pl.BlockSpec(memory_space=pl.ANY)
    out, _ = pl.pallas_call(
        kernel,
        in_specs=[any_spec] * 6,
        out_specs=[any_spec, any_spec],
        out_shape=[
            jax.ShapeDtypeStruct((N, C), x.dtype),
            jax.ShapeDtypeStruct((T - S - len(DROP), F // 128, TM, 128), _BF),
        ],
        scratch_shapes=[
            pltpu.VMEM((NX, TM, C), _BF),
            pltpu.VMEM((2, SUB1, C), _BF),
            pltpu.VMEM((S, F // 128, TM, 128), _BF),
            pltpu.VMEM((C, F), _BF),
            pltpu.VMEM((F, C), _BF),
            pltpu.VMEM((60, 64, 128), _U32),
            pltpu.VMEM((60, 64, 128), _U32),
            pltpu.VMEM((_NP, SUB1 // 4, 128), _U32),
            pltpu.VMEM((max(PLA, 1) * _NP, SUB1 // 2, 128), _F32),
            pltpu.VMEM((8, F), _F32),
            pltpu.VMEM((8, C), _F32),
            pltpu.VMEM((1, 1, C), _BF),
            pltpu.VMEM((F,), _BF),
            pltpu.VMEM((F,), _BF),
            pltpu.SemaphoreType.DMA((NX,)),
            pltpu.SemaphoreType.DMA((2,)),
            pltpu.SemaphoreType.DMA((NX,)),
            pltpu.SemaphoreType.DMA((S,)),
            pltpu.SemaphoreType.DMA((5,)),
        ],
        compiler_params=pltpu.CompilerParams(
            vmem_limit_bytes=VMEM_MB * 1024 * 1024,
            disable_bounds_checks=bool(NOBC),
        ),
    )(x2, dw, w1, w2, grn_g, grn_b)
    return out.reshape(B, H, W, C)


@jax.jit
def pallas_standalone__modern_conv_block_slak__vision_kernel(
    x: jax.Array,
    dw: jax.Array,
    w1: jax.Array,
    w2: jax.Array,
    grn_g: jax.Array,
    grn_b: jax.Array,
):
    return _run(x, dw, w1, w2, grn_g, grn_b)
```

```python
import math

import jax
import jax.numpy as jnp
import jax.experimental.pallas as pl
import jax.experimental.pallas.tpu as pltpu

_LN_EPS = 1e-5
_GRN_EPS = 1e-6
_GA = 2.0 * math.sqrt(2.0 / math.pi)
_GB = 8.0 * math.sqrt(2.0 / math.pi) * 0.044715
_ALPHA = _GB ** (-1.0 / 3.0)
_GZ = _GA * _ALPHA
_KT = 128
_BF = jnp.bfloat16
_F32 = jnp.float32
_U32 = jnp.uint32

_HK_U = (
    ((1, 1, 1),),
    ((1, 0, 0), (1, 1, 1)),
    ((1, 0, 0), (-1, 1, 0), (1, 1, 2)),
    ((1, 0, 1), (-1, 0, 2), (-1, 1, 1), (1, 1, 2)),
    ((1, 1, 0), (1, 1, 1)),
    ((1, 0, 1), (-1, 0, 2), (-1, 1, 1)),
    ((1, 1, 0), (-1, 0, 0)),
    ((1, 0, 2),),
    ((1, 0, 1), (-1, 0, 2)),
    ((1, 1, 2),),
    ((1, 0, 2), (-1, 0, 0), (1, 1, 0), (-1, 1, 2)),
    ((1, 0, 0), (1, 0, 1)),
    ((1, 1, 0), (-1, 1, 2)),
    ((1, 1, 1), (-1, 0, 1)),
    ((1, 0, 0),),
)
_NP = len(_HK_U)


def _hk_a(a11, a12, a13, a21, a22, a23):
    d1 = a12 - a13
    d2 = d1 - a22
    e1 = a21 - a23
    l2 = a11 - e1
    return (a22, a11 + a22, l2, d2 + a23, a21 + a22, d2, a21 - a11, a13, d1, a23,
            a13 - l2, a11 + a12, e1, a22 - a12, a11)


def _hk_b(b):
    return (
        b(2, 3) - b(1, 3) - b(2, 2),
        b(1, 3) - b(2, 1),
        b(1, 2) - b(3, 1),
        b(3, 3),
        b(1, 3),
        -b(2, 2) - b(3, 3),
        b(1, 1) - b(1, 3) + b(3, 1),
        b(2, 2) + b(3, 1) + b(3, 2),
        b(2, 2),
        b(1, 2) + b(3, 2) - b(3, 3),
        b(3, 1),
        b(2, 1),
        b(1, 2),
        b(2, 1) - b(2, 3) - b(3, 3),
        b(1, 1) + b(1, 2) - b(2, 1),
    )


def _hk_c(P, emit):
    q8 = P(8)
    a = P(5) + q8
    b = a + P(3)
    p0 = P(0)
    p4 = P(4)
    emit(1, 2, b + p0 + p4)
    a = a + p0
    p12 = P(12)
    emit(1, 1, b + P(9) + p12)
    d = P(2) + p12
    p10 = P(10)
    emit(0, 1, d + q8 + P(7) - p10)
    e = P(14) - d
    p11 = P(11)
    emit(0, 0, e + p10 + p11)
    p1 = P(1)
    emit(0, 2, a + p11 + p1 + P(13))
    emit(1, 0, e + p4 - p1 + P(6))


def _pack(v):
    return pltpu.bitcast(v.astype(_BF), _U32)


def _unpack(u):
    return pltpu.bitcast(u, _BF)


def _dot(a, b):
    return jnp.dot(a, b, preferred_element_type=_F32)


def _make_kernel(*, T, TM, C, F, S, NX, SUB1, SUB2, RB, DROP, PRIO, PLA=2):
    KT = _KT
    H1 = SUB1 // 2
    H2 = SUB2 // 2
    NCH = TM // SUB2
    NS1 = TM // SUB1
    N3 = F // (3 * KT)

    def inc_mod(v, m):
        return jnp.where(v + 1 == m, 0, v + 1)

    def dec_mod(v, m):
        return jnp.where(v == 0, m - 1, v - 1)

    def kept(t):
        k = t >= 0
        for d in DROP:
            k = jnp.logical_and(k, t != d)
        return k

    def hidx(t):
        i = t
        for d in DROP:
            i = i - (t > d).astype(jnp.int32)
        return i

    def kernel(x_hbm, dw_hbm, w1_hbm, w2_hbm, g_hbm, b_hbm,
               o_hbm, hbuf_hbm,
               xv, xh, hv, w1v, w2v, wc1, wc2, lk, pk, acc_ref, bias_ref, dwv, gv, bv,
               xsem, xhsem, osem, hsem, wsem):

        def x_copy(tile, s):
            return pltpu.make_async_copy(x_hbm.at[pl.ds(tile * TM, TM)], xv.at[s], xsem.at[s])

        def xh_copy(tile, s):
            return pltpu.make_async_copy(x_hbm.at[pl.ds(tile * TM, SUB1)], xh.at[s], xhsem.at[s])

        def o_copy(tile, s, c):
            r = c * SUB2
            return pltpu.make_async_copy(xv.at[s, pl.ds(r, SUB2)],
                                         o_hbm.at[pl.ds(tile * TM + r, SUB2)], osem.at[s])

        def h_write(tile, slot):
            return pltpu.make_async_copy(hv.at[slot], hbuf_hbm.at[hidx(tile)], hsem.at[slot])

        def h_read(tile, slot, c):
            rows = pl.ds(c * SUB2, SUB2)
            return pltpu.make_async_copy(hbuf_hbm.at[hidx(tile), :, rows, :],
                                         hv.at[slot, :, rows, :], hsem.at[slot])

        w1_copy = pltpu.make_async_copy(w1_hbm, w1v, wsem.at[0])
        w2_copy = pltpu.make_async_copy(w2_hbm, w2v, wsem.at[1])
        dw_copy = pltpu.make_async_copy(dw_hbm, dwv, wsem.at[2])
        g_copy = pltpu.make_async_copy(g_hbm, gv, wsem.at[3])
        b_copy = pltpu.make_async_copy(b_hbm, bv, wsem.at[4])

        dw_copy.start()
        xh_copy(0, 0).start()
        w1_copy.start()
        xh_copy(1, 1).start()
        x_copy(0, 0).start()

        acc_ref[...] = jnp.zeros_like(acc_ref)

        w1_copy.wait()
        for q in range(N3):
            b = lambda l, j: w1v[(l - 1) * KT:l * KT,
                                 ((j - 1) * N3 + q) * KT:((j - 1) * N3 + q + 1) * KT].astype(_F32)
            for i, cmb in enumerate(_hk_b(b)):
                wc1[i * N3 + q] = _pack(cmb)

        dw_copy.wait()
        dw = dwv[0].astype(_F32)

        def prep(xs):
            xs = xs.astype(_F32) * dw
            m = jnp.mean(xs, axis=-1, keepdims=True)
            xc = xs - m
            ssq = jnp.sum(xc * xc, axis=-1, keepdims=True)
            xn = xc * jnp.exp(math.log(0.5 * math.sqrt(C) / _ALPHA)
                              - 0.5 * jnp.log(ssq + C * _LN_EPS))
            blocks = [xn[i * H1:(i + 1) * H1, l * KT:(l + 1) * KT] for i in range(2) for l in range(3)]
            return [o.astype(_BF) for o in _hk_a(*blocks)]

        def lookahead(xs):
            L = prep(xs)
            for i, o in enumerate(L):
                lk[i] = pltpu.bitcast(o, _U32)
            for q in range(PLA):
                for i in range(_NP):
                    pk[q * _NP + i] = _dot(L[i], _unpack(wc1[i * N3 + q]))

        def hidden_rows(L, slot, r0, stats, pre=0):
            for q in range(N3):
                part = {}

                def emit(i, j, z):
                    g = z + z * jnp.tanh(z * (_GZ + z * z))
                    ct = j * N3 + q
                    if stats:
                        gg = jnp.sum((g * g).reshape(H1 // 8, 8, KT), axis=0)
                        if j not in part:
                            part[j] = gg
                        else:
                            acc_ref[:, ct * KT:(ct + 1) * KT] += gg + part[j]
                    hv[slot, ct, pl.ds(r0 + i * H1, H1), :] = g.astype(_BF)

                if q < pre:
                    _hk_c(lambda i: pk[q * _NP + i], emit)
                else:
                    _hk_c(lambda i: _dot(L[i], _unpack(wc1[i * N3 + q])), emit)

        xh_copy(0, 0).wait()
        lookahead(xh[0])
        x_copy(0, 0).wait()
        x_copy(1, 1).start()
        w2_copy.start(priority=PRIO)
        g_copy.start()
        b_copy.start()

        def phase0(t, carry):
            slot, xs_cur, hs_nxt = carry
            xs_n1 = inc_mod(xs_cur, NX)
            xs_n2 = inc_mod(xs_n1, NX)

            @pl.when(t > 0)
            def _():
                x_copy(t, xs_cur).wait()

            @pl.when(t + 1 < T)
            def _():
                xh_copy(t + 1, hs_nxt).wait()

            @pl.when(t + 2 < T)
            def _():
                x_copy(t + 2, xs_n2).start()
                xh_copy(t + 2, 1 - hs_nxt).start()

            @pl.when(jnp.logical_and(t >= S, kept(t - S)))
            def _():
                h_write(t - S, slot).wait()

            for si in range(NS1):
                r0 = si * SUB1
                if si == 0:
                    L = [_unpack(lk[i]) for i in range(_NP)]
                else:
                    L = prep(xv[xs_cur, r0:r0 + SUB1, :])
                hidden_rows(L, slot, r0, True, PLA if si == 0 else 0)

            lookahead(xh[hs_nxt])

            @pl.when(jnp.logical_and(t < T - S, kept(t)))
            def _():
                h_write(t, slot).start(priority=PRIO)

            return inc_mod(slot, S), xs_n1, 1 - hs_nxt

        i32 = jnp.int32
        jax.lax.fori_loop(0, T, phase0, (i32(0), i32(0), i32(1)))

        w2_copy.wait()
        g_copy.wait()
        b_copy.wait()
        ss = jnp.sum(acc_ref[...], axis=0, keepdims=True)
        gx = jnp.sqrt(ss * (_ALPHA * _ALPHA) + _GRN_EPS)
        nx = gx / (jnp.mean(gx, axis=-1, keepdims=True) + _GRN_EPS)
        s = (gv[...].reshape(1, F).astype(_F32) * nx + 1.0) * _ALPHA
        st = jnp.transpose(jnp.broadcast_to(s, (128, F)))
        F3 = F // 3
        b = lambda l, j: (w2v[(l - 1) * F3:l * F3, (j - 1) * KT:j * KT].astype(_F32)
                          * st[(l - 1) * F3:l * F3])
        for i, cmb in enumerate(_hk_b(b)):
            for q in range(N3):
                wc2[i * N3 + q] = _pack(cmb[q * KT:(q + 1) * KT, :])
        bb = jnp.broadcast_to(bv[...].reshape(1, F), (16, F))
        bias_ref[...] = _dot(bb, w2v[...])[:8]

        def phase1(j, carry):
            tile = T - 1 - j
            slot, xs_cur = carry
            xs_nxt = dec_mod(xs_cur, NX)

            @pl.when(jnp.logical_and(j >= S, kept(tile)))
            def _():
                for c in range(NCH):
                    h_read(tile, slot, c).wait()

            @pl.when(j >= NX)
            def _():
                x_copy(tile, xs_cur).wait()

            @pl.when(j >= 2)
            def _():
                xs_p2 = inc_mod(inc_mod(xs_cur, NX), NX)
                for c in range(NCH):
                    o_copy(tile + 2, xs_p2, c).wait()

                @pl.when(tile + 2 >= NX)
                def _():
                    x_copy(tile + 2 - NX, xs_p2).start()

            if DROP:
                @pl.when(jnp.logical_not(kept(tile)))
                def _():
                    def stash(rr):
                        for i, o in enumerate(prep(xv[xs_cur, pl.ds(rr, SUB1), :])):
                            lk[i] = pltpu.bitcast(o, _U32)

                    stash(0)

                    def body(k, c):
                        r0 = pl.multiple_of(k * RB, RB)
                        for si in range(RB // SUB1):
                            rr = pl.multiple_of(r0 + si * SUB1, SUB1)
                            if si == 0:
                                L = [_unpack(lk[i]) for i in range(_NP)]
                            else:
                                L = prep(xv[xs_cur, pl.ds(rr, SUB1), :])
                            hidden_rows(L, slot, rr, False)
                        stash(pl.multiple_of(jnp.minimum(r0 + RB, TM - RB), RB))
                        return c
                    jax.lax.fori_loop(0, TM // RB, body, 0)

            bias = bias_ref[0:1, :]
            for si in range(NCH):
                r0 = si * SUB2

                def op(r, terms):
                    sl = slot + jax.lax.shift_right_logical(j, 16 + r)
                    pc = lambda i, l, q: hv[sl, l * N3 + q, r0 + i * H2:r0 + (i + 1) * H2, :]
                    if len(terms) == 1:
                        _, i, l = terms[0]
                        return jnp.concatenate([pc(i, l, q) for q in range(N3)], axis=1)
                    acc = None
                    for sg, i, l in terms:
                        v = jnp.concatenate([pc(i, l, q).astype(_F32) for q in range(N3)], axis=1)
                        acc = v if acc is None else (acc + v if sg > 0 else acc - v)
                    return acc.astype(_BF)

                ops = [op(r, _HK_U[r]) for r in range(_NP)]

                def emit(i, jn, y):
                    rows = slice(r0 + i * H2, r0 + (i + 1) * H2)
                    cols = slice(jn * KT, (jn + 1) * KT)
                    y = y + bias[:, cols] + xv[xs_cur, rows, cols].astype(_F32)
                    xv[xs_cur, rows, cols] = y.astype(xv.dtype)

                _hk_c(lambda i: _dot(ops[i], _unpack(
                    wc2[i * N3:(i + 1) * N3].reshape(N3 * (KT // 2), KT))), emit)

                o_copy(tile, xs_cur, si).start()

                @pl.when(jnp.logical_and(tile >= S, kept(tile - S)))
                def _():
                    h_read(tile - S, slot, si).start(priority=PRIO)

            return dec_mod(slot, S), xs_nxt

        jax.lax.fori_loop(0, T, phase1, (i32((T - 1) % S), i32((T - 1) % NX)))

        for tile in (1, 0):
            for c in range(NCH):
                o_copy(tile, tile % NX, c).wait()

    return kernel


def _run(x, dw, w1, w2, grn_g, grn_b, *, TM=3072, S=12, NX=3, SUB1=128, SUB2=1024, RB=1024,
         D1=31, D2=17, D3=-1, VMEM_MB=128, PRIO=1, NOBC=1, PLA=2):
    B, H, W, C = x.shape
    F = w1.shape[1]
    N = B * H * W
    T = N // TM
    DROP = tuple(d for d in (D1, D2, D3) if d >= 0)
    assert N % TM == 0 and T > S and T >= NX and all(d < T - S for d in DROP)

    x2 = x.reshape(N, C)
    kernel = _make_kernel(T=T, TM=TM, C=C, F=F, S=S, NX=NX, SUB1=SUB1, SUB2=SUB2, RB=RB,
                          DROP=DROP, PRIO=PRIO, PLA=PLA)
    any_spec = pl.BlockSpec(memory_space=pl.ANY)
    out, _ = pl.pallas_call(
        kernel,
        in_specs=[any_spec] * 6,
        out_specs=[any_spec, any_spec],
        out_shape=[
            jax.ShapeDtypeStruct((N, C), x.dtype),
            jax.ShapeDtypeStruct((T - S - len(DROP), F // 128, TM, 128), _BF),
        ],
        scratch_shapes=[
            pltpu.VMEM((NX, TM, C), _BF),
            pltpu.VMEM((2, SUB1, C), _BF),
            pltpu.VMEM((S, F // 128, TM, 128), _BF),
            pltpu.VMEM((C, F), _BF),
            pltpu.VMEM((F, C), _BF),
            pltpu.VMEM((60, 64, 128), _U32),
            pltpu.VMEM((60, 64, 128), _U32),
            pltpu.VMEM((_NP, SUB1 // 4, 128), _U32),
            pltpu.VMEM((max(PLA, 1) * _NP, SUB1 // 2, 128), _F32),
            pltpu.VMEM((8, F), _F32),
            pltpu.VMEM((8, C), _F32),
            pltpu.VMEM((1, 1, C), _BF),
            pltpu.VMEM((F,), _BF),
            pltpu.VMEM((F,), _BF),
            pltpu.SemaphoreType.DMA((NX,)),
            pltpu.SemaphoreType.DMA((2,)),
            pltpu.SemaphoreType.DMA((NX,)),
            pltpu.SemaphoreType.DMA((S,)),
            pltpu.SemaphoreType.DMA((5,)),
        ],
        compiler_params=pltpu.CompilerParams(
            vmem_limit_bytes=VMEM_MB * 1024 * 1024,
            disable_bounds_checks=bool(NOBC),
        ),
    )(x2, dw, w1, w2, grn_g, grn_b)
    return out.reshape(B, H, W, C)


@jax.jit
def pallas_standalone__modern_conv_block_slak__vision_kernel(
    x: jax.Array,
    dw: jax.Array,
    w1: jax.Array,
    w2: jax.Array,
    grn_g: jax.Array,
    grn_b: jax.Array,
):
    return _run(x, dw, w1, w2, grn_g, grn_b)
```

```python
import math

import jax
import jax.numpy as jnp
import jax.experimental.pallas as pl
import jax.experimental.pallas.tpu as pltpu

_LN_EPS = 1e-5
_GRN_EPS = 1e-6
_GA = 2.0 * math.sqrt(2.0 / math.pi)
_GB = 8.0 * math.sqrt(2.0 / math.pi) * 0.044715
_ALPHA = _GB ** (-1.0 / 3.0)
_GZ = _GA * _ALPHA
_KT = 128
_BF = jnp.bfloat16
_F32 = jnp.float32
_U32 = jnp.uint32

_HK_U = (
    ((1, 1, 1),),
    ((1, 0, 0), (1, 1, 1)),
    ((1, 0, 0), (-1, 1, 0), (1, 1, 2)),
    ((1, 0, 1), (-1, 0, 2), (-1, 1, 1), (1, 1, 2)),
    ((1, 1, 0), (1, 1, 1)),
    ((1, 0, 1), (-1, 0, 2), (-1, 1, 1)),
    ((1, 1, 0), (-1, 0, 0)),
    ((1, 0, 2),),
    ((1, 0, 1), (-1, 0, 2)),
    ((1, 1, 2),),
    ((1, 0, 2), (-1, 0, 0), (1, 1, 0), (-1, 1, 2)),
    ((1, 0, 0), (1, 0, 1)),
    ((1, 1, 0), (-1, 1, 2)),
    ((1, 1, 1), (-1, 0, 1)),
    ((1, 0, 0),),
)
_NP = len(_HK_U)


def _hk_a(a11, a12, a13, a21, a22, a23):
    d1 = a12 - a13
    d2 = d1 - a22
    e1 = a21 - a23
    l2 = a11 - e1
    return (a22, a11 + a22, l2, d2 + a23, a21 + a22, d2, a21 - a11, a13, d1, a23,
            a13 - l2, a11 + a12, e1, a22 - a12, a11)


def _hk_b(b):
    return (
        b(2, 3) - b(1, 3) - b(2, 2),
        b(1, 3) - b(2, 1),
        b(1, 2) - b(3, 1),
        b(3, 3),
        b(1, 3),
        -b(2, 2) - b(3, 3),
        b(1, 1) - b(1, 3) + b(3, 1),
        b(2, 2) + b(3, 1) + b(3, 2),
        b(2, 2),
        b(1, 2) + b(3, 2) - b(3, 3),
        b(3, 1),
        b(2, 1),
        b(1, 2),
        b(2, 1) - b(2, 3) - b(3, 3),
        b(1, 1) + b(1, 2) - b(2, 1),
    )


def _hk_c(P, emit):
    p12 = P(12)
    d = P(2) + p12
    p10 = P(10)
    q8 = P(8)
    emit(0, 1, (P(7) - p10) + (d + q8))
    e = P(14) - d
    p11 = P(11)
    emit(0, 0, (e + p10) + p11)
    p1 = P(1)
    p4 = P(4)
    emit(1, 0, (e - p1) + (p4 + P(6)))
    a = P(5) + q8
    p0 = P(0)
    emit(0, 2, (p11 + p1) + (a + p0) + P(13))
    b = a + P(3)
    emit(1, 2, (p0 + p4) + b)
    emit(1, 1, (P(9) + p12) + b)


def _hk_c2(P, emit):
    q8 = P(8)
    a = P(5) + q8
    b = a + P(3)
    p0 = P(0)
    p4 = P(4)
    emit(1, 2, b + p0 + p4)
    a = a + p0
    p12 = P(12)
    emit(1, 1, b + P(9) + p12)
    d = P(2) + p12
    p10 = P(10)
    emit(0, 1, d + q8 + P(7) - p10)
    e = P(14) - d
    p11 = P(11)
    emit(0, 0, e + p10 + p11)
    p1 = P(1)
    emit(0, 2, a + p11 + p1 + P(13))
    emit(1, 0, e + p4 - p1 + P(6))


def _pack(v):
    return pltpu.bitcast(v.astype(_BF), _U32)


def _unpack(u):
    return pltpu.bitcast(u, _BF)


def _dot(a, b):
    return jnp.dot(a, b, preferred_element_type=_F32)


def _make_kernel(*, T, TM, C, F, S, NX, SUB1, SUB2, RB, DROP, PRIO, PLA=2):
    KT = _KT
    H1 = SUB1 // 2
    H2 = SUB2 // 2
    NCH = TM // SUB2
    NS1 = TM // SUB1
    N3 = F // (3 * KT)

    def inc_mod(v, m):
        return jnp.where(v + 1 == m, 0, v + 1)

    def dec_mod(v, m):
        return jnp.where(v == 0, m - 1, v - 1)

    def kept(t):
        k = t >= 0
        for d in DROP:
            k = jnp.logical_and(k, t != d)
        return k

    def hidx(t):
        i = t
        for d in DROP:
            i = i - (t > d).astype(jnp.int32)
        return i

    def kernel(x_hbm, dw_hbm, w1_hbm, w2_hbm, g_hbm, b_hbm,
               o_hbm, hbuf_hbm,
               xv, xh, hv, w1v, w2v, wc1, wc2, lk, pk, acc_ref, bias_ref, dwv, gv, bv,
               xsem, xhsem, osem, hsem, wsem):

        def x_copy(tile, s):
            return pltpu.make_async_copy(x_hbm.at[pl.ds(tile * TM, TM)], xv.at[s], xsem.at[s])

        def xh_copy(tile, s):
            return pltpu.make_async_copy(x_hbm.at[pl.ds(tile * TM, SUB1)], xh.at[s], xhsem.at[s])

        def o_copy(tile, s, c):
            r = c * SUB2
            return pltpu.make_async_copy(xv.at[s, pl.ds(r, SUB2)],
                                         o_hbm.at[pl.ds(tile * TM + r, SUB2)], osem.at[s])

        def h_write(tile, slot):
            return pltpu.make_async_copy(hv.at[slot], hbuf_hbm.at[hidx(tile)], hsem.at[slot])

        def h_read(tile, slot, c):
            rows = pl.ds(c * SUB2, SUB2)
            return pltpu.make_async_copy(hbuf_hbm.at[hidx(tile), :, rows, :],
                                         hv.at[slot, :, rows, :], hsem.at[slot])

        w1_copy = pltpu.make_async_copy(w1_hbm, w1v, wsem.at[0])
        w2_copy = pltpu.make_async_copy(w2_hbm, w2v, wsem.at[1])
        dw_copy = pltpu.make_async_copy(dw_hbm, dwv, wsem.at[2])
        g_copy = pltpu.make_async_copy(g_hbm, gv, wsem.at[3])
        b_copy = pltpu.make_async_copy(b_hbm, bv, wsem.at[4])

        dw_copy.start()
        xh_copy(0, 0).start()
        w1_copy.start()
        xh_copy(1, 1).start()
        x_copy(0, 0).start()

        acc_ref[...] = jnp.zeros_like(acc_ref)

        w1_copy.wait()
        for q in range(N3):
            b = lambda l, j: w1v[(l - 1) * KT:l * KT,
                                 ((j - 1) * N3 + q) * KT:((j - 1) * N3 + q + 1) * KT].astype(_F32)
            for i, cmb in enumerate(_hk_b(b)):
                wc1[i * N3 + q] = _pack(cmb)

        dw_copy.wait()
        dw = dwv[0].astype(_F32)

        def prep(xs):
            xs = xs.astype(_F32) * dw
            m = jnp.mean(xs, axis=-1, keepdims=True)
            xc = xs - m
            ssq = jnp.sum(xc * xc, axis=-1, keepdims=True)
            xn = xc * jnp.exp(math.log(0.5 * math.sqrt(C) / _ALPHA)
                              - 0.5 * jnp.log(ssq + C * _LN_EPS))
            blocks = [xn[i * H1:(i + 1) * H1, l * KT:(l + 1) * KT] for i in range(2) for l in range(3)]
            return [o.astype(_BF) for o in _hk_a(*blocks)]

        def lookahead(xs):
            L = prep(xs)
            for i, o in enumerate(L):
                lk[i] = pltpu.bitcast(o, _U32)
            for q in range(PLA):
                for i in range(_NP):
                    pk[q * _NP + i] = _dot(L[i], _unpack(wc1[i * N3 + q]))

        def hidden_rows(L, slot, r0, stats, pre=0):
            for q in range(N3):
                part = {}

                def emit(i, j, z):
                    g = z * (1.0 + jnp.tanh(z * (_GZ + z * z)))
                    ct = j * N3 + q
                    if stats:
                        gg = jnp.sum((g * g).reshape(H1 // 8, 8, KT), axis=0)
                        if j not in part:
                            part[j] = gg
                        else:
                            acc_ref[:, ct * KT:(ct + 1) * KT] += gg + part[j]
                    hv[slot, ct, pl.ds(r0 + i * H1, H1), :] = g.astype(_BF)

                if q < pre:
                    _hk_c(lambda i: pk[q * _NP + i], emit)
                else:
                    _hk_c(lambda i: _dot(L[i], _unpack(wc1[i * N3 + q])), emit)

        xh_copy(0, 0).wait()
        lookahead(xh[0])
        x_copy(0, 0).wait()
        x_copy(1, 1).start()
        w2_copy.start(priority=PRIO)
        g_copy.start()
        b_copy.start()

        def phase0(t, carry):
            slot, xs_cur, hs_nxt = carry
            xs_n1 = inc_mod(xs_cur, NX)
            xs_n2 = inc_mod(xs_n1, NX)

            @pl.when(t > 0)
            def _():
                x_copy(t, xs_cur).wait()

            @pl.when(t + 1 < T)
            def _():
                xh_copy(t + 1, hs_nxt).wait()

            @pl.when(t + 2 < T)
            def _():
                x_copy(t + 2, xs_n2).start()
                xh_copy(t + 2, 1 - hs_nxt).start()

            @pl.when(jnp.logical_and(t >= S, kept(t - S)))
            def _():
                h_write(t - S, slot).wait()

            for si in range(NS1):
                r0 = si * SUB1
                if si == 0:
                    L = [_unpack(lk[i]) for i in range(_NP)]
                else:
                    L = prep(xv[xs_cur, r0:r0 + SUB1, :])
                hidden_rows(L, slot, r0, True, PLA if si == 0 else 0)

            lookahead(xh[hs_nxt])

            @pl.when(jnp.logical_and(t < T - S, kept(t)))
            def _():
                h_write(t, slot).start(priority=PRIO)

            return inc_mod(slot, S), xs_n1, 1 - hs_nxt

        i32 = jnp.int32
        jax.lax.fori_loop(0, T, phase0, (i32(0), i32(0), i32(1)))

        w2_copy.wait()
        g_copy.wait()
        b_copy.wait()
        ss = jnp.sum(acc_ref[...], axis=0, keepdims=True)
        gx = jnp.sqrt(ss * (_ALPHA * _ALPHA) + _GRN_EPS)
        nx = gx / (jnp.mean(gx, axis=-1, keepdims=True) + _GRN_EPS)
        s = (gv[...].reshape(1, F).astype(_F32) * nx + 1.0) * _ALPHA
        st = jnp.transpose(jnp.broadcast_to(s, (128, F)))
        F3 = F // 3
        b = lambda l, j: (w2v[(l - 1) * F3:l * F3, (j - 1) * KT:j * KT].astype(_F32)
                          * st[(l - 1) * F3:l * F3])
        for i, cmb in enumerate(_hk_b(b)):
            for q in range(N3):
                wc2[i * N3 + q] = _pack(cmb[q * KT:(q + 1) * KT, :])
        bb = jnp.broadcast_to(bv[...].reshape(1, F), (16, F))
        bias_ref[...] = _dot(bb, w2v[...])[:8]

        def phase1(j, carry):
            tile = T - 1 - j
            slot, xs_cur = carry
            xs_nxt = dec_mod(xs_cur, NX)

            @pl.when(jnp.logical_and(j >= S, kept(tile)))
            def _():
                for c in range(NCH):
                    h_read(tile, slot, c).wait()

            @pl.when(j >= NX)
            def _():
                x_copy(tile, xs_cur).wait()

            @pl.when(j >= 2)
            def _():
                xs_p2 = inc_mod(inc_mod(xs_cur, NX), NX)
                for c in range(NCH):
                    o_copy(tile + 2, xs_p2, c).wait()

                @pl.when(tile + 2 >= NX)
                def _():
                    x_copy(tile + 2 - NX, xs_p2).start()

            if DROP:
                @pl.when(jnp.logical_not(kept(tile)))
                def _():
                    def stash(rr):
                        for i, o in enumerate(prep(xv[xs_cur, pl.ds(rr, SUB1), :])):
                            lk[i] = pltpu.bitcast(o, _U32)

                    stash(0)

                    def body(k, c):
                        r0 = pl.multiple_of(k * RB, RB)
                        for si in range(RB // SUB1):
                            rr = pl.multiple_of(r0 + si * SUB1, SUB1)
                            if si == 0:
                                L = [_unpack(lk[i]) for i in range(_NP)]
                            else:
                                L = prep(xv[xs_cur, pl.ds(rr, SUB1), :])
                            hidden_rows(L, slot, rr, False)
                        stash(pl.multiple_of(jnp.minimum(r0 + RB, TM - RB), RB))
                        return c
                    jax.lax.fori_loop(0, TM // RB, body, 0)

            bias = bias_ref[0:1, :]
            for si in range(NCH):
                r0 = si * SUB2

                def op(r, terms):
                    sl = slot + jax.lax.shift_right_logical(j, 16 + r)
                    pc = lambda i, l, q: hv[sl, l * N3 + q, r0 + i * H2:r0 + (i + 1) * H2, :]
                    if len(terms) == 1:
                        _, i, l = terms[0]
                        return jnp.concatenate([pc(i, l, q) for q in range(N3)], axis=1)
                    acc = None
                    for sg, i, l in terms:
                        v = jnp.concatenate([pc(i, l, q).astype(_F32) for q in range(N3)], axis=1)
                        acc = v if acc is None else (acc + v if sg > 0 else acc - v)
                    return acc.astype(_BF)

                ops = [op(r, _HK_U[r]) for r in range(_NP)]

                def emit(i, jn, y):
                    rows = slice(r0 + i * H2, r0 + (i + 1) * H2)
                    cols = slice(jn * KT, (jn + 1) * KT)
                    y = y + bias[:, cols] + xv[xs_cur, rows, cols].astype(_F32)
                    xv[xs_cur, rows, cols] = y.astype(xv.dtype)

                _hk_c2(lambda i: _dot(ops[i], _unpack(
                    wc2[i * N3:(i + 1) * N3].reshape(N3 * (KT // 2), KT))), emit)

                o_copy(tile, xs_cur, si).start()

                @pl.when(jnp.logical_and(tile >= S, kept(tile - S)))
                def _():
                    h_read(tile - S, slot, si).start(priority=PRIO)

            return dec_mod(slot, S), xs_nxt

        jax.lax.fori_loop(0, T, phase1, (i32((T - 1) % S), i32((T - 1) % NX)))

        for tile in (1, 0):
            for c in range(NCH):
                o_copy(tile, tile % NX, c).wait()

    return kernel


def _run(x, dw, w1, w2, grn_g, grn_b, *, TM=3072, S=12, NX=3, SUB1=128, SUB2=1024, RB=1024,
         D1=31, D2=17, D3=-1, VMEM_MB=128, PRIO=1, NOBC=1, PLA=2):
    B, H, W, C = x.shape
    F = w1.shape[1]
    N = B * H * W
    T = N // TM
    DROP = tuple(d for d in (D1, D2, D3) if d >= 0)
    assert N % TM == 0 and T > S and T >= NX and all(d < T - S for d in DROP)

    x2 = x.reshape(N, C)
    kernel = _make_kernel(T=T, TM=TM, C=C, F=F, S=S, NX=NX, SUB1=SUB1, SUB2=SUB2, RB=RB,
                          DROP=DROP, PRIO=PRIO, PLA=PLA)
    any_spec = pl.BlockSpec(memory_space=pl.ANY)
    out, _ = pl.pallas_call(
        kernel,
        in_specs=[any_spec] * 6,
        out_specs=[any_spec, any_spec],
        out_shape=[
            jax.ShapeDtypeStruct((N, C), x.dtype),
            jax.ShapeDtypeStruct((T - S - len(DROP), F // 128, TM, 128), _BF),
        ],
        scratch_shapes=[
            pltpu.VMEM((NX, TM, C), _BF),
            pltpu.VMEM((2, SUB1, C), _BF),
            pltpu.VMEM((S, F // 128, TM, 128), _BF),
            pltpu.VMEM((C, F), _BF),
            pltpu.VMEM((F, C), _BF),
            pltpu.VMEM((60, 64, 128), _U32),
            pltpu.VMEM((60, 64, 128), _U32),
            pltpu.VMEM((_NP, SUB1 // 4, 128), _U32),
            pltpu.VMEM((max(PLA, 1) * _NP, SUB1 // 2, 128), _F32),
            pltpu.VMEM((8, F), _F32),
            pltpu.VMEM((8, C), _F32),
            pltpu.VMEM((1, 1, C), _BF),
            pltpu.VMEM((F,), _BF),
            pltpu.VMEM((F,), _BF),
            pltpu.SemaphoreType.DMA((NX,)),
            pltpu.SemaphoreType.DMA((2,)),
            pltpu.SemaphoreType.DMA((NX,)),
            pltpu.SemaphoreType.DMA((S,)),
            pltpu.SemaphoreType.DMA((5,)),
        ],
        compiler_params=pltpu.CompilerParams(
            vmem_limit_bytes=VMEM_MB * 1024 * 1024,
            disable_bounds_checks=bool(NOBC),
        ),
    )(x2, dw, w1, w2, grn_g, grn_b)
    return out.reshape(B, H, W, C)


@jax.jit
def pallas_standalone__modern_conv_block_slak__vision_kernel(
    x: jax.Array,
    dw: jax.Array,
    w1: jax.Array,
    w2: jax.Array,
    grn_g: jax.Array,
    grn_b: jax.Array,
):
    return _run(x, dw, w1, w2, grn_g, grn_b)
```

```python
import math

import jax
import jax.numpy as jnp
import jax.experimental.pallas as pl
import jax.experimental.pallas.tpu as pltpu

_LN_EPS = 1e-5
_GRN_EPS = 1e-6
_GA = 2.0 * math.sqrt(2.0 / math.pi)
_GB = 8.0 * math.sqrt(2.0 / math.pi) * 0.044715
_ALPHA = _GB ** (-1.0 / 3.0)
_GZ = _GA * _ALPHA
_KT = 128
_BF = jnp.bfloat16
_F32 = jnp.float32
_U32 = jnp.uint32

_HK_U = (
    ((1, 1, 1),),
    ((1, 0, 0), (1, 1, 1)),
    ((1, 0, 0), (-1, 1, 0), (1, 1, 2)),
    ((1, 0, 1), (-1, 0, 2), (-1, 1, 1), (1, 1, 2)),
    ((1, 1, 0), (1, 1, 1)),
    ((1, 0, 1), (-1, 0, 2), (-1, 1, 1)),
    ((1, 1, 0), (-1, 0, 0)),
    ((1, 0, 2),),
    ((1, 0, 1), (-1, 0, 2)),
    ((1, 1, 2),),
    ((1, 0, 2), (-1, 0, 0), (1, 1, 0), (-1, 1, 2)),
    ((1, 0, 0), (1, 0, 1)),
    ((1, 1, 0), (-1, 1, 2)),
    ((1, 1, 1), (-1, 0, 1)),
    ((1, 0, 0),),
)
_NP = len(_HK_U)


def _hk_a(a11, a12, a13, a21, a22, a23):
    d1 = a12 - a13
    d2 = d1 - a22
    e1 = a21 - a23
    l2 = a11 - e1
    return (a22, a11 + a22, l2, d2 + a23, a21 + a22, d2, a21 - a11, a13, d1, a23,
            a13 - l2, a11 + a12, e1, a22 - a12, a11)


def _hk_b(b):
    return (
        b(2, 3) - b(1, 3) - b(2, 2),
        b(1, 3) - b(2, 1),
        b(1, 2) - b(3, 1),
        b(3, 3),
        b(1, 3),
        -b(2, 2) - b(3, 3),
        b(1, 1) - b(1, 3) + b(3, 1),
        b(2, 2) + b(3, 1) + b(3, 2),
        b(2, 2),
        b(1, 2) + b(3, 2) - b(3, 3),
        b(3, 1),
        b(2, 1),
        b(1, 2),
        b(2, 1) - b(2, 3) - b(3, 3),
        b(1, 1) + b(1, 2) - b(2, 1),
    )


def _hk_c(P, emit):
    p12 = P(12)
    d = P(2) + p12
    p10 = P(10)
    q8 = P(8)
    emit(0, 1, (P(7) - p10) + (d + q8))
    e = P(14) - d
    p11 = P(11)
    emit(0, 0, (e + p10) + p11)
    p1 = P(1)
    p4 = P(4)
    emit(1, 0, (e - p1) + (p4 + P(6)))
    a = P(5) + q8
    p0 = P(0)
    emit(0, 2, (p11 + p1) + (a + p0) + P(13))
    b = a + P(3)
    emit(1, 2, (p0 + p4) + b)
    emit(1, 1, (P(9) + p12) + b)


def _hk_c2(P, emit):
    q8 = P(8)
    a = P(5) + q8
    b = a + P(3)
    p0 = P(0)
    p4 = P(4)
    emit(1, 2, b + p0 + p4)
    a = a + p0
    p12 = P(12)
    emit(1, 1, b + P(9) + p12)
    d = P(2) + p12
    p10 = P(10)
    emit(0, 1, d + q8 + P(7) - p10)
    e = P(14) - d
    p11 = P(11)
    emit(0, 0, e + p10 + p11)
    p1 = P(1)
    emit(0, 2, a + p11 + p1 + P(13))
    emit(1, 0, e + p4 - p1 + P(6))


def _pack(v):
    return pltpu.bitcast(v.astype(_BF), _U32)


def _unpack(u):
    return pltpu.bitcast(u, _BF)


def _dot(a, b):
    return jnp.dot(a, b, preferred_element_type=_F32)


def _make_kernel(*, T, TM, C, F, S, NX, SUB1, SUB2, RB, RECOMP, PRIO, PLA=2):
    KT = _KT
    H1 = SUB1 // 2
    H2 = SUB2 // 2
    NCH = TM // SUB2
    NS1 = TM // SUB1
    N3 = F // (3 * KT)

    def inc_mod(v, m):
        return jnp.where(v + 1 == m, 0, v + 1)

    def dec_mod(v, m):
        return jnp.where(v == 0, m - 1, v - 1)

    def spilled(t):
        k = t >= 0
        for d in RECOMP:
            k = jnp.logical_and(k, t != d)
        return k

    def hidx(t):
        i = t
        for d in RECOMP:
            i = i - (t > d).astype(jnp.int32)
        return i

    def kernel(x_hbm, dw_hbm, w1_hbm, w2_hbm, g_hbm, b_hbm,
               o_hbm, hbuf_hbm,
               xv, xh, hv, w1v, w2v, wc1, wc2, lk, pk, acc_ref, bias_ref, dwv, gv, bv,
               xsem, xhsem, osem, hsem, wsem):

        def x_copy(tile, s):
            return pltpu.make_async_copy(x_hbm.at[pl.ds(tile * TM, TM)], xv.at[s], xsem.at[s])

        def xh_copy(tile, s):
            return pltpu.make_async_copy(x_hbm.at[pl.ds(tile * TM, SUB1)], xh.at[s], xhsem.at[s])

        def o_copy(tile, s, c):
            r = c * SUB2
            return pltpu.make_async_copy(xv.at[s, pl.ds(r, SUB2)],
                                         o_hbm.at[pl.ds(tile * TM + r, SUB2)], osem.at[s])

        def h_write(tile, slot):
            return pltpu.make_async_copy(hv.at[slot], hbuf_hbm.at[hidx(tile)], hsem.at[slot])

        def h_read(tile, slot, c):
            rows = pl.ds(c * SUB2, SUB2)
            return pltpu.make_async_copy(hbuf_hbm.at[hidx(tile), :, rows, :],
                                         hv.at[slot, :, rows, :], hsem.at[slot])

        w1_copy = pltpu.make_async_copy(w1_hbm, w1v, wsem.at[0])
        w2_copy = pltpu.make_async_copy(w2_hbm, w2v, wsem.at[1])
        dw_copy = pltpu.make_async_copy(dw_hbm, dwv, wsem.at[2])
        g_copy = pltpu.make_async_copy(g_hbm, gv, wsem.at[3])
        b_copy = pltpu.make_async_copy(b_hbm, bv, wsem.at[4])

        dw_copy.start()
        xh_copy(0, 0).start()
        w1_copy.start()
        xh_copy(1, 1).start()
        x_copy(0, 0).start()

        acc_ref[...] = jnp.zeros_like(acc_ref)

        w1_copy.wait()
        for q in range(N3):
            b = lambda l, j: w1v[(l - 1) * KT:l * KT,
                                 ((j - 1) * N3 + q) * KT:((j - 1) * N3 + q + 1) * KT].astype(_F32)
            for i, cmb in enumerate(_hk_b(b)):
                wc1[i * N3 + q] = _pack(cmb)

        dw_copy.wait()
        dw = dwv[0].astype(_F32)

        def prep(xs):
            xs = xs.astype(_F32) * dw
            m = jnp.mean(xs, axis=-1, keepdims=True)
            xc = xs - m
            ssq = jnp.sum(xc * xc, axis=-1, keepdims=True)
            xn = xc * jnp.exp(math.log(0.5 * math.sqrt(C) / _ALPHA)
                              - 0.5 * jnp.log(ssq + C * _LN_EPS))
            blocks = [xn[i * H1:(i + 1) * H1, l * KT:(l + 1) * KT] for i in range(2) for l in range(3)]
            return [o.astype(_BF) for o in _hk_a(*blocks)]

        def lookahead(xs):
            L = prep(xs)
            for i, o in enumerate(L):
                lk[i] = pltpu.bitcast(o, _U32)
            for q in range(PLA):
                for i in range(_NP):
                    pk[q * _NP + i] = _dot(L[i], _unpack(wc1[i * N3 + q]))

        def hidden_rows(L, slot, r0, stats, pre=0):
            for q in range(N3):
                part = {}

                def emit(i, j, z):
                    g = z * (1.0 + jnp.tanh(z * (_GZ + z * z)))
                    ct = j * N3 + q
                    if stats:
                        gg = jnp.sum((g * g).reshape(H1 // 8, 8, KT), axis=0)
                        if j not in part:
                            part[j] = gg
                        else:
                            acc_ref[:, ct * KT:(ct + 1) * KT] += gg + part[j]
                    hv[slot, ct, pl.ds(r0 + i * H1, H1), :] = g.astype(_BF)

                if q < pre:
                    _hk_c(lambda i: pk[q * _NP + i], emit)
                else:
                    _hk_c(lambda i: _dot(L[i], _unpack(wc1[i * N3 + q])), emit)

        xh_copy(0, 0).wait()
        lookahead(xh[0])
        x_copy(0, 0).wait()
        x_copy(1, 1).start()
        w2_copy.start(priority=PRIO)
        g_copy.start()
        b_copy.start()

        def phase0(t, carry):
            slot, xs_cur, hs_nxt = carry
            xs_n1 = inc_mod(xs_cur, NX)
            xs_n2 = inc_mod(xs_n1, NX)

            @pl.when(t > 0)
            def _():
                x_copy(t, xs_cur).wait()

            @pl.when(t + 1 < T)
            def _():
                xh_copy(t + 1, hs_nxt).wait()

            @pl.when(t + 2 < T)
            def _():
                x_copy(t + 2, xs_n2).start()
                xh_copy(t + 2, 1 - hs_nxt).start()

            @pl.when(jnp.logical_and(t >= S, spilled(t - S)))
            def _():
                h_write(t - S, slot).wait()

            for si in range(NS1):
                r0 = si * SUB1
                if si == 0:
                    L = [_unpack(lk[i]) for i in range(_NP)]
                else:
                    L = prep(xv[xs_cur, r0:r0 + SUB1, :])
                hidden_rows(L, slot, r0, True, PLA if si == 0 else 0)

            lookahead(xh[hs_nxt])

            @pl.when(jnp.logical_and(t < T - S, spilled(t)))
            def _():
                h_write(t, slot).start(priority=PRIO)

            return inc_mod(slot, S), xs_n1, 1 - hs_nxt

        i32 = jnp.int32
        jax.lax.fori_loop(0, T, phase0, (i32(0), i32(0), i32(1)))

        w2_copy.wait()
        g_copy.wait()
        b_copy.wait()
        ss = jnp.sum(acc_ref[...], axis=0, keepdims=True)
        gx = jnp.sqrt(ss * (_ALPHA * _ALPHA) + _GRN_EPS)
        nx = gx / (jnp.mean(gx, axis=-1, keepdims=True) + _GRN_EPS)
        s = (gv[...].reshape(1, F).astype(_F32) * nx + 1.0) * _ALPHA
        st = jnp.transpose(jnp.broadcast_to(s, (128, F)))
        F3 = F // 3
        b = lambda l, j: (w2v[(l - 1) * F3:l * F3, (j - 1) * KT:j * KT].astype(_F32)
                          * st[(l - 1) * F3:l * F3])
        for i, cmb in enumerate(_hk_b(b)):
            for q in range(N3):
                wc2[i * N3 + q] = _pack(cmb[q * KT:(q + 1) * KT, :])
        bb = jnp.broadcast_to(bv[...].reshape(1, F), (16, F))
        bias_ref[...] = _dot(bb, w2v[...])[:8]

        def phase1(j, carry):
            tile = T - 1 - j
            slot, xs_cur = carry
            xs_nxt = dec_mod(xs_cur, NX)

            @pl.when(jnp.logical_and(j >= S, spilled(tile)))
            def _():
                for c in range(NCH):
                    h_read(tile, slot, c).wait()

            @pl.when(j >= NX)
            def _():
                x_copy(tile, xs_cur).wait()

            @pl.when(j >= 2)
            def _():
                xs_p2 = inc_mod(inc_mod(xs_cur, NX), NX)
                for c in range(NCH):
                    o_copy(tile + 2, xs_p2, c).wait()

                @pl.when(tile + 2 >= NX)
                def _():
                    x_copy(tile + 2 - NX, xs_p2).start()

            if RECOMP:
                @pl.when(jnp.logical_not(spilled(tile)))
                def _():
                    def stash(rr):
                        for i, o in enumerate(prep(xv[xs_cur, pl.ds(rr, SUB1), :])):
                            lk[i] = pltpu.bitcast(o, _U32)

                    stash(0)

                    def body(k, c):
                        r0 = pl.multiple_of(k * RB, RB)
                        for si in range(RB // SUB1):
                            rr = pl.multiple_of(r0 + si * SUB1, SUB1)
                            if si == 0:
                                L = [_unpack(lk[i]) for i in range(_NP)]
                            else:
                                L = prep(xv[xs_cur, pl.ds(rr, SUB1), :])
                            hidden_rows(L, slot, rr, False)
                        stash(pl.multiple_of(jnp.minimum(r0 + RB, TM - RB), RB))
                        return c
                    jax.lax.fori_loop(0, TM // RB, body, 0)

            bias = bias_ref[0:1, :]
            for si in range(NCH):
                r0 = si * SUB2

                def op(r, terms):
                    sl = slot + jax.lax.shift_right_logical(j, 16 + r)
                    pc = lambda i, l, q: hv[sl, l * N3 + q, r0 + i * H2:r0 + (i + 1) * H2, :]
                    if len(terms) == 1:
                        _, i, l = terms[0]
                        return jnp.concatenate([pc(i, l, q) for q in range(N3)], axis=1)
                    acc = None
                    for sg, i, l in terms:
                        v = jnp.concatenate([pc(i, l, q).astype(_F32) for q in range(N3)], axis=1)
                        acc = v if acc is None else (acc + v if sg > 0 else acc - v)
                    return acc.astype(_BF)

                ops = [op(r, _HK_U[r]) for r in range(_NP)]

                def emit(i, jn, y):
                    rows = slice(r0 + i * H2, r0 + (i + 1) * H2)
                    cols = slice(jn * KT, (jn + 1) * KT)
                    y = y + bias[:, cols] + xv[xs_cur, rows, cols].astype(_F32)
                    xv[xs_cur, rows, cols] = y.astype(xv.dtype)

                _hk_c2(lambda i: _dot(ops[i], _unpack(
                    wc2[i * N3:(i + 1) * N3].reshape(N3 * (KT // 2), KT))), emit)

                o_copy(tile, xs_cur, si).start()

                @pl.when(jnp.logical_and(tile >= S, spilled(tile - S)))
                def _():
                    h_read(tile - S, slot, si).start(priority=PRIO)

            return dec_mod(slot, S), xs_nxt

        jax.lax.fori_loop(0, T, phase1, (i32((T - 1) % S), i32((T - 1) % NX)))

        for tile in (1, 0):
            for c in range(NCH):
                o_copy(tile, tile % NX, c).wait()

    return kernel


def _run(x, dw, w1, w2, grn_g, grn_b, *, TM=3072, S=12, NX=3, SUB1=128, SUB2=1024, RB=1024,
         R1=31, R2=17, VMEM_MB=128, PRIO=1, NOBC=1, PLA=2):
    B, H, W, C = x.shape
    F = w1.shape[1]
    N = B * H * W
    T = N // TM
    RECOMP = tuple(d for d in (R1, R2) if d >= 0)
    assert N % TM == 0 and T > S and T >= NX and all(d < T - S for d in RECOMP)

    x2 = x.reshape(N, C)
    kernel = _make_kernel(T=T, TM=TM, C=C, F=F, S=S, NX=NX, SUB1=SUB1, SUB2=SUB2, RB=RB,
                          RECOMP=RECOMP, PRIO=PRIO, PLA=PLA)
    any_spec = pl.BlockSpec(memory_space=pl.ANY)
    out, _ = pl.pallas_call(
        kernel,
        in_specs=[any_spec] * 6,
        out_specs=[any_spec, any_spec],
        out_shape=[
            jax.ShapeDtypeStruct((N, C), x.dtype),
            jax.ShapeDtypeStruct((T - S - len(RECOMP), F // 128, TM, 128), _BF),
        ],
        scratch_shapes=[
            pltpu.VMEM((NX, TM, C), _BF),
            pltpu.VMEM((2, SUB1, C), _BF),
            pltpu.VMEM((S, F // 128, TM, 128), _BF),
            pltpu.VMEM((C, F), _BF),
            pltpu.VMEM((F, C), _BF),
            pltpu.VMEM((60, 64, 128), _U32),
            pltpu.VMEM((60, 64, 128), _U32),
            pltpu.VMEM((_NP, SUB1 // 4, 128), _U32),
            pltpu.VMEM((max(PLA, 1) * _NP, SUB1 // 2, 128), _F32),
            pltpu.VMEM((8, F), _F32),
            pltpu.VMEM((8, C), _F32),
            pltpu.VMEM((1, 1, C), _BF),
            pltpu.VMEM((F,), _BF),
            pltpu.VMEM((F,), _BF),
            pltpu.SemaphoreType.DMA((NX,)),
            pltpu.SemaphoreType.DMA((2,)),
            pltpu.SemaphoreType.DMA((NX,)),
            pltpu.SemaphoreType.DMA((S,)),
            pltpu.SemaphoreType.DMA((5,)),
        ],
        compiler_params=pltpu.CompilerParams(
            vmem_limit_bytes=VMEM_MB * 1024 * 1024,
            disable_bounds_checks=bool(NOBC),
        ),
    )(x2, dw, w1, w2, grn_g, grn_b)
    return out.reshape(B, H, W, C)


@jax.jit
def pallas_standalone__modern_conv_block_slak__vision_kernel(
    x: jax.Array,
    dw: jax.Array,
    w1: jax.Array,
    w2: jax.Array,
    grn_g: jax.Array,
    grn_b: jax.Array,
):
    return _run(x, dw, w1, w2, grn_g, grn_b)
```

```python
import math

import jax
import jax.numpy as jnp
import jax.experimental.pallas as pl
import jax.experimental.pallas.tpu as pltpu

_LN_EPS = 1e-5
_GRN_EPS = 1e-6
_GA = 2.0 * math.sqrt(2.0 / math.pi)
_GB = 8.0 * math.sqrt(2.0 / math.pi) * 0.044715
_ALPHA = _GB ** (-1.0 / 3.0)
_GZ = _GA * _ALPHA
_KT = 128
_BF = jnp.bfloat16
_F32 = jnp.float32
_U32 = jnp.uint32

_HK_U = (
    ((1, 1, 1),),
    ((1, 0, 0), (1, 1, 1)),
    ((1, 0, 0), (-1, 1, 0), (1, 1, 2)),
    ((1, 0, 1), (-1, 0, 2), (-1, 1, 1), (1, 1, 2)),
    ((1, 1, 0), (1, 1, 1)),
    ((1, 0, 1), (-1, 0, 2), (-1, 1, 1)),
    ((1, 1, 0), (-1, 0, 0)),
    ((1, 0, 2),),
    ((1, 0, 1), (-1, 0, 2)),
    ((1, 1, 2),),
    ((1, 0, 2), (-1, 0, 0), (1, 1, 0), (-1, 1, 2)),
    ((1, 0, 0), (1, 0, 1)),
    ((1, 1, 0), (-1, 1, 2)),
    ((1, 1, 1), (-1, 0, 1)),
    ((1, 0, 0),),
)
_NP = len(_HK_U)


def _hk_a(a11, a12, a13, a21, a22, a23):
    d1 = a12 - a13
    d2 = d1 - a22
    e1 = a21 - a23
    l2 = a11 - e1
    return (a22, a11 + a22, l2, d2 + a23, a21 + a22, d2, a21 - a11, a13, d1, a23,
            a13 - l2, a11 + a12, e1, a22 - a12, a11)


def _hk_b(b):
    return (
        b(2, 3) - b(1, 3) - b(2, 2),
        b(1, 3) - b(2, 1),
        b(1, 2) - b(3, 1),
        b(3, 3),
        b(1, 3),
        -b(2, 2) - b(3, 3),
        b(1, 1) - b(1, 3) + b(3, 1),
        b(2, 2) + b(3, 1) + b(3, 2),
        b(2, 2),
        b(1, 2) + b(3, 2) - b(3, 3),
        b(3, 1),
        b(2, 1),
        b(1, 2),
        b(2, 1) - b(2, 3) - b(3, 3),
        b(1, 1) + b(1, 2) - b(2, 1),
    )


def _hk_c(P, emit):
    p12 = P(12)
    d = P(2) + p12
    p10 = P(10)
    q8 = P(8)
    emit(0, 1, (P(7) - p10) + (d + q8))
    e = P(14) - d
    p11 = P(11)
    emit(0, 0, (e + p10) + p11)
    p1 = P(1)
    p4 = P(4)
    emit(1, 0, (e - p1) + (p4 + P(6)))
    a = P(5) + q8
    p0 = P(0)
    emit(0, 2, (p11 + p1) + (a + p0) + P(13))
    b = a + P(3)
    emit(1, 2, (p0 + p4) + b)
    emit(1, 1, (P(9) + p12) + b)


def _hk_c2(P, emit):
    q8 = P(8)
    a = P(5) + q8
    b = a + P(3)
    p0 = P(0)
    p4 = P(4)
    emit(1, 2, b + p0 + p4)
    a = a + p0
    p12 = P(12)
    emit(1, 1, b + P(9) + p12)
    d = P(2) + p12
    p10 = P(10)
    emit(0, 1, d + q8 + P(7) - p10)
    e = P(14) - d
    p11 = P(11)
    emit(0, 0, e + p10 + p11)
    p1 = P(1)
    emit(0, 2, a + p11 + p1 + P(13))
    emit(1, 0, e + p4 - p1 + P(6))


def _pack(v):
    return pltpu.bitcast(v.astype(_BF), _U32)


def _unpack(u):
    return pltpu.bitcast(u, _BF)


def _dot(a, b):
    return jnp.dot(a, b, preferred_element_type=_F32)


def _make_kernel(*, T, TM, C, F, S, NX, SUB1, SUB2, RECOMP, PART, RC, PRIO, PLA=2):
    KT = _KT
    H1 = SUB1 // 2
    H2 = SUB2 // 2
    NCH = TM // SUB2
    NS1 = TM // SUB1
    N3 = F // (3 * KT)

    def inc_mod(v, m):
        return jnp.where(v + 1 == m, 0, v + 1)

    def dec_mod(v, m):
        return jnp.where(v == 0, m - 1, v - 1)

    def spilled(t):
        k = t != PART
        for d in RECOMP:
            k = jnp.logical_and(k, t != d)
        return k

    def hidx(t):
        i = t - (t > PART).astype(jnp.int32)
        for d in RECOMP:
            i = i - (t > d).astype(jnp.int32)
        return i

    def kernel(x_hbm, dw_hbm, w1_hbm, w2_hbm, g_hbm, b_hbm,
               o_hbm, hbuf_hbm, hbuf2_hbm,
               xv, xh, hv, w2v, wc1, wc2, lk, pk, acc_ref, bias_ref, dwv, gv, bv,
               xsem, xhsem, osem, hsem, wsem):

        def x_copy(tile, s):
            return pltpu.make_async_copy(x_hbm.at[pl.ds(tile * TM, TM)], xv.at[s], xsem.at[s])

        def xh_copy(tile, s):
            return pltpu.make_async_copy(x_hbm.at[pl.ds(tile * TM, SUB1)], xh.at[s], xhsem.at[s])

        def o_copy(tile, s, c):
            r = c * SUB2
            return pltpu.make_async_copy(xv.at[s, pl.ds(r, SUB2)],
                                         o_hbm.at[pl.ds(tile * TM + r, SUB2)], osem.at[s])

        def o_copy_tile(tile, s):
            return pltpu.make_async_copy(xv.at[s], o_hbm.at[pl.ds(tile * TM, TM)], osem.at[s])

        def h_write(tile, slot):
            return pltpu.make_async_copy(hv.at[slot], hbuf_hbm.at[hidx(tile)], hsem.at[slot])

        def h_read(tile, slot, c):
            rows = pl.ds(c * SUB2, SUB2)
            return pltpu.make_async_copy(hbuf_hbm.at[hidx(tile), :, rows, :],
                                         hv.at[slot, :, rows, :], hsem.at[slot])

        def part_rows(slot):
            return hv.at[slot, :, pl.ds(RC * SUB2, TM - RC * SUB2), :]

        def hp_write(slot):
            return pltpu.make_async_copy(part_rows(slot), hbuf2_hbm, hsem.at[slot])

        def hp_read(slot):
            return pltpu.make_async_copy(hbuf2_hbm, part_rows(slot), hsem.at[slot])

        w1_copies = [pltpu.make_async_copy(w1_hbm.at[:, pl.ds(ct * KT, KT)],
                                           hv.at[S - 1, ct, pl.ds(0, C), :], wsem.at[0])
                     for ct in range(F // KT)]
        w2_copy = pltpu.make_async_copy(w2_hbm, w2v, wsem.at[1])
        dw_copy = pltpu.make_async_copy(dw_hbm, dwv, wsem.at[2])
        g_copy = pltpu.make_async_copy(g_hbm, gv, wsem.at[3])
        b_copy = pltpu.make_async_copy(b_hbm, bv, wsem.at[4])

        dw_copy.start()
        xh_copy(0, 0).start()
        for cp in w1_copies:
            cp.start()
        xh_copy(1, 1).start()
        x_copy(0, 0).start()

        acc_ref[...] = jnp.zeros_like(acc_ref)

        for cp in w1_copies:
            cp.wait()
        for q in range(N3):
            b = lambda l, j: hv[S - 1, (j - 1) * N3 + q, (l - 1) * KT:l * KT, :].astype(_F32)
            for i, cmb in enumerate(_hk_b(b)):
                wc1[i * N3 + q] = _pack(cmb)

        dw_copy.wait()
        dw = dwv[0].astype(_F32)

        def prep(xs):
            xs = xs.astype(_F32) * dw
            m = jnp.mean(xs, axis=-1, keepdims=True)
            xc = xs - m
            ssq = jnp.sum(xc * xc, axis=-1, keepdims=True)
            xn = xc * jnp.exp(math.log(0.5 * math.sqrt(C) / _ALPHA)
                              - 0.5 * jnp.log(ssq + C * _LN_EPS))
            blocks = [xn[i * H1:(i + 1) * H1, l * KT:(l + 1) * KT] for i in range(2) for l in range(3)]
            return [o.astype(_BF) for o in _hk_a(*blocks)]

        def lookahead(xs):
            L = prep(xs)
            for i, o in enumerate(L):
                lk[i] = pltpu.bitcast(o, _U32)
            for q in range(PLA):
                for i in range(_NP):
                    pk[q * _NP + i] = _dot(L[i], _unpack(wc1[i * N3 + q]))

        def hidden_rows(L, slot, r0, stats, pre=0):
            for q in range(N3):
                part = {}

                def emit(i, j, z):
                    g = z * (1.0 + jnp.tanh(z * (_GZ + z * z)))
                    ct = j * N3 + q
                    if stats:
                        gg = jnp.sum((g * g).reshape(H1 // 8, 8, KT), axis=0)
                        if j not in part:
                            part[j] = gg
                        else:
                            acc_ref[:, ct * KT:(ct + 1) * KT] += gg + part[j]
                    hv[slot, ct, pl.ds(r0 + i * H1, H1), :] = g.astype(_BF)

                if q < pre:
                    _hk_c(lambda i: pk[q * _NP + i], emit)
                else:
                    _hk_c(lambda i: _dot(L[i], _unpack(wc1[i * N3 + q])), emit)

        xh_copy(0, 0).wait()
        lookahead(xh[0])
        x_copy(0, 0).wait()
        x_copy(1, 1).start()
        w2_copy.start(priority=PRIO)
        g_copy.start()
        b_copy.start()

        def phase0(t, carry):
            slot, xs_cur, hs_nxt = carry
            xs_n1 = inc_mod(xs_cur, NX)
            xs_n2 = inc_mod(xs_n1, NX)

            @pl.when(t > 0)
            def _():
                x_copy(t, xs_cur).wait()

            @pl.when(t + 1 < T)
            def _():
                xh_copy(t + 1, hs_nxt).wait()

            @pl.when(t + 2 < T)
            def _():
                x_copy(t + 2, xs_n2).start()
                xh_copy(t + 2, 1 - hs_nxt).start()

            @pl.when(jnp.logical_and(t >= S, spilled(t - S)))
            def _():
                h_write(t - S, slot).wait()

            @pl.when(t - S == PART)
            def _():
                hp_write(slot).wait()

            for si in range(NS1):
                r0 = si * SUB1
                if si == 0:
                    L = [_unpack(lk[i]) for i in range(_NP)]
                else:
                    L = prep(xv[xs_cur, r0:r0 + SUB1, :])
                hidden_rows(L, slot, r0, True, PLA if si == 0 else 0)

            lookahead(xh[hs_nxt])

            @pl.when(jnp.logical_and(t < T - S, spilled(t)))
            def _():
                h_write(t, slot).start(priority=PRIO)

            @pl.when(t == PART)
            def _():
                hp_write(slot).start(priority=PRIO)

            return inc_mod(slot, S), xs_n1, 1 - hs_nxt

        i32 = jnp.int32
        jax.lax.fori_loop(0, T, phase0, (i32(0), i32(0), i32(1)))

        w2_copy.wait()
        g_copy.wait()
        b_copy.wait()
        ss = jnp.sum(acc_ref[...], axis=0, keepdims=True)
        gx = jnp.sqrt(ss * (_ALPHA * _ALPHA) + _GRN_EPS)
        nx = gx / (jnp.mean(gx, axis=-1, keepdims=True) + _GRN_EPS)
        s = (gv[...].reshape(1, F).astype(_F32) * nx + 1.0) * _ALPHA
        st = jnp.transpose(jnp.broadcast_to(s, (128, F)))
        F3 = F // 3
        b = lambda l, j: (w2v[(l - 1) * F3:l * F3, (j - 1) * KT:j * KT].astype(_F32)
                          * st[(l - 1) * F3:l * F3])
        for i, cmb in enumerate(_hk_b(b)):
            for q in range(N3):
                wc2[i * N3 + q] = _pack(cmb[q * KT:(q + 1) * KT, :])
        bb = jnp.broadcast_to(bv[...].reshape(1, F), (16, F))
        bias_ref[...] = _dot(bb, w2v[...])[:8]

        def phase1(j, carry):
            tile = T - 1 - j
            slot, xs_cur = carry
            xs_nxt = dec_mod(xs_cur, NX)

            @pl.when(jnp.logical_and(j >= S, spilled(tile)))
            def _():
                for c in range(NCH):
                    h_read(tile, slot, c).wait()

            @pl.when(tile == PART)
            def _():
                hp_read(slot).wait()

            @pl.when(j >= NX)
            def _():
                x_copy(tile, xs_cur).wait()

            @pl.when(j >= 2)
            def _():
                xs_p2 = inc_mod(inc_mod(xs_cur, NX), NX)
                o_copy_tile(tile + 2, xs_p2).wait()

                @pl.when(tile + 2 >= NX)
                def _():
                    x_copy(tile + 2 - NX, xs_p2).start()

            @pl.when(jnp.logical_not(spilled(tile)))
            def _():
                def stash(rr):
                    for i, o in enumerate(prep(xv[xs_cur, pl.ds(rr, SUB1), :])):
                        lk[i] = pltpu.bitcast(o, _U32)

                stash(0)

                def body(k, c):
                    r0 = pl.multiple_of(k * SUB2, SUB2)
                    for si in range(SUB2 // SUB1):
                        rr = pl.multiple_of(r0 + si * SUB1, SUB1)
                        if si == 0:
                            L = [_unpack(lk[i]) for i in range(_NP)]
                        else:
                            L = prep(xv[xs_cur, pl.ds(rr, SUB1), :])
                        hidden_rows(L, slot, rr, False)
                    stash(pl.multiple_of(jnp.minimum(r0 + SUB2, TM - SUB2), SUB2))
                    return c
                jax.lax.fori_loop(0, jnp.where(tile == PART, RC, NCH), body, 0)

            bias = bias_ref[0:1, :]
            for si in range(NCH):
                r0 = si * SUB2

                def op(r, terms):
                    sl = slot + jax.lax.shift_right_logical(j, 16 + r)
                    pc = lambda i, l, q: hv[sl, l * N3 + q, r0 + i * H2:r0 + (i + 1) * H2, :]
                    if len(terms) == 1:
                        _, i, l = terms[0]
                        return jnp.concatenate([pc(i, l, q) for q in range(N3)], axis=1)
                    acc = None
                    for sg, i, l in terms:
                        v = jnp.concatenate([pc(i, l, q).astype(_F32) for q in range(N3)], axis=1)
                        acc = v if acc is None else (acc + v if sg > 0 else acc - v)
                    return acc.astype(_BF)

                ops = [op(r, _HK_U[r]) for r in range(_NP)]

                def emit(i, jn, y):
                    rows = slice(r0 + i * H2, r0 + (i + 1) * H2)
                    cols = slice(jn * KT, (jn + 1) * KT)
                    y = y + bias[:, cols] + xv[xs_cur, rows, cols].astype(_F32)
                    xv[xs_cur, rows, cols] = y.astype(xv.dtype)

                _hk_c2(lambda i: _dot(ops[i], _unpack(
                    wc2[i * N3:(i + 1) * N3].reshape(N3 * (KT // 2), KT))), emit)

                @pl.when(tile == 0)
                def _():
                    o_copy(tile, xs_cur, si).start()

                @pl.when(jnp.logical_and(tile >= S, spilled(tile - S)))
                def _():
                    h_read(tile - S, slot, si).start(priority=PRIO)

            @pl.when(tile - S == PART)
            def _():
                hp_read(slot).start(priority=PRIO)

            @pl.when(tile > 0)
            def _():
                o_copy_tile(tile, xs_cur).start()

            return dec_mod(slot, S), xs_nxt

        jax.lax.fori_loop(0, T, phase1, (i32((T - 1) % S), i32((T - 1) % NX)))

        o_copy_tile(1, 1 % NX).wait()
        for c in range(NCH):
            o_copy(0, 0, c).wait()

    return kernel


def _run(x, dw, w1, w2, grn_g, grn_b, *, TM=3072, S=12, NX=4, SUB1=128, SUB2=1024,
         R1=31, PART=17, RC=2, VMEM_MB=128, PRIO=1, NOBC=1, PLA=2):
    B, H, W, C = x.shape
    F = w1.shape[1]
    N = B * H * W
    T = N // TM
    NCH = TM // SUB2
    RECOMP = (R1,)
    assert N % TM == 0 and T > S and T >= NX and max(R1, PART) < T - S and R1 != PART
    assert 0 < RC < NCH

    x2 = x.reshape(N, C)
    kernel = _make_kernel(T=T, TM=TM, C=C, F=F, S=S, NX=NX, SUB1=SUB1, SUB2=SUB2,
                          RECOMP=RECOMP, PART=PART, RC=RC, PRIO=PRIO, PLA=PLA)
    any_spec = pl.BlockSpec(memory_space=pl.ANY)
    out, _, _ = pl.pallas_call(
        kernel,
        in_specs=[any_spec] * 6,
        out_specs=[any_spec, any_spec, any_spec],
        out_shape=[
            jax.ShapeDtypeStruct((N, C), x.dtype),
            jax.ShapeDtypeStruct((T - S - len(RECOMP) - 1, F // 128, TM, 128), _BF),
            jax.ShapeDtypeStruct((F // 128, TM - RC * SUB2, 128), _BF),
        ],
        scratch_shapes=[
            pltpu.VMEM((NX, TM, C), _BF),
            pltpu.VMEM((2, SUB1, C), _BF),
            pltpu.VMEM((S, F // 128, TM, 128), _BF),
            pltpu.VMEM((F, C), _BF),
            pltpu.VMEM((60, 64, 128), _U32),
            pltpu.VMEM((60, 64, 128), _U32),
            pltpu.VMEM((_NP, SUB1 // 4, 128), _U32),
            pltpu.VMEM((max(PLA, 1) * _NP, SUB1 // 2, 128), _F32),
            pltpu.VMEM((8, F), _F32),
            pltpu.VMEM((8, C), _F32),
            pltpu.VMEM((1, 1, C), _BF),
            pltpu.VMEM((F,), _BF),
            pltpu.VMEM((F,), _BF),
            pltpu.SemaphoreType.DMA((NX,)),
            pltpu.SemaphoreType.DMA((2,)),
            pltpu.SemaphoreType.DMA((NX,)),
            pltpu.SemaphoreType.DMA((S,)),
            pltpu.SemaphoreType.DMA((5,)),
        ],
        compiler_params=pltpu.CompilerParams(
            vmem_limit_bytes=VMEM_MB * 1024 * 1024,
            disable_bounds_checks=bool(NOBC),
        ),
    )(x2, dw, w1, w2, grn_g, grn_b)
    return out.reshape(B, H, W, C)


@jax.jit
def pallas_standalone__modern_conv_block_slak__vision_kernel(
    x: jax.Array,
    dw: jax.Array,
    w1: jax.Array,
    w2: jax.Array,
    grn_g: jax.Array,
    grn_b: jax.Array,
):
    return _run(x, dw, w1, w2, grn_g, grn_b)
```
